```python
import os as _os
_os.environ.setdefault("JAX_PLATFORMS", "cpu")
import jax
import jax.numpy as jnp

def _softmax(x, axis=-1):
    return jax.nn.softmax(x, axis=axis)
def _gelu(x):
    return jax.nn.gelu(x, approximate=True)
def _silu(x):
    return jax.nn.silu(x)
def _sigmoid(x):
    return jax.nn.sigmoid(x)
def _layernorm(x, axis=-1, eps=1e-5):
    m = jnp.mean(x, axis=axis, keepdims=True)
    v = jnp.var(x, axis=axis, keepdims=True)
    return (x - m) / jnp.sqrt(v + eps)
def _scatter_add(tgt, idx, src, axis=0):
    return tgt.at[idx].add(src)
def _segment_sum(src, seg, n):
    return jax.ops.segment_sum(src, seg, n)
class _Rng:
    def __init__(self, key):
        self._k = key
    def _next(self):
        self._k, sub = jax.random.split(self._k)
        return sub
    def normal(self, shape):
        return jax.random.normal(self._next(), shape, dtype=jnp.bfloat16)
    def randint(self, lo, hi, shape):
        return jax.random.randint(self._next(), shape, lo, hi, dtype=jnp.int32)
    def uniform(self, shape, lo=0.0, hi=1.0):
        return jax.random.uniform(self._next(), shape, jnp.bfloat16, lo, hi)
    def permutation(self, n):
        return jax.random.permutation(self._next(), n)


kernel_name = 'interleave_layers__softmax_full_mha__glu_gated_bilinear__prompt'

def setup_inputs():
    _rng = _Rng(jax.random.key(int.from_bytes(__import__("os").urandom(4), "little")))
    _w = (lambda a: (lambda t: t.astype(jnp.bfloat16) if jnp.issubdtype(t.dtype, jnp.floating) else t)(jnp.asarray(a)))
    def _A_setup():
        B, S, D = 1, 2048, 512
        return {
            "x": _w((lambda *s: _rng.normal(s) * 0.05)(B, S, D)),
            "wqkv": _w((lambda *s: _rng.normal(s) * 0.05)(D, 3 * D)),
            "wo": _w((lambda *s: _rng.normal(s) * 0.05)(D, D)),
        }
    _A_in = _A_setup()

    def _B_setup():
        B, S, D, F = 1, 2048, 512, 1792
        return {
            "x": _w((lambda *s: _rng.normal(s) * 0.05)(B, S, D)),
            "w_gate": _w((lambda *s: _rng.normal(s) * 0.4)(D, F) * (D ** -0.5)),
            "w_up": _w((lambda *s: _rng.normal(s) * 0.4)(D, F) * (D ** -0.5)),
            "w_down": _w((lambda *s: _rng.normal(s) * 0.4)(F, D) * (F ** -0.5)),
        }
    _B_in = _B_setup()

    return {
        "A_x": _A_in["x"],
        "A_wqkv": _A_in["wqkv"],
        "A_wo": _A_in["wo"],
        "B_x": _B_in["x"],
        "B_w_gate": _B_in["w_gate"],
        "B_w_up": _B_in["w_up"],
        "B_w_down": _B_in["w_down"],
    }

def reference(A_x, A_wqkv, A_wo, B_x, B_w_gate, B_w_up, B_w_down):
    def _A_ref(x, wqkv, wo):
        B, S, D = x.shape
        H = 32; Dh = D // H
        qkv = (lambda x, *d: x.transpose(*d))((x @ wqkv).reshape(B, S, 3, H, Dh), 2, 0, 3, 1, 4)
        q, k, v = qkv[0], qkv[1], qkv[2]
        scale = Dh ** -0.5
        scores = jnp.einsum("bhqd,bhkd->bhqk", q, k) * scale
        p = _softmax(scores, axis=-1)
        o = jnp.einsum("bhqk,bhkd->bhqd", p, v)
        return (lambda x, *d: x.transpose(*d))(o, 0, 2, 1, 3).reshape(B, S, D) @ wo

    def _B_ref(x, w_gate, w_up, w_down):
        g = jnp.einsum("bsd,df->bsf", x, w_gate)
        u = jnp.einsum("bsd,df->bsf", x, w_up)
        h = g * u
        return jnp.einsum("bsf,fd->bsd", h, w_down)

    x = A_x
    x = x + _A_ref(_layernorm(x, axis=-1), A_wqkv, A_wo)
    x = x + _B_ref(_layernorm(x, axis=-1), B_w_gate, B_w_up, B_w_down)
    x = x + _A_ref(_layernorm(x, axis=-1), A_wqkv, A_wo)
    x = x + _B_ref(_layernorm(x, axis=-1), B_w_gate, B_w_up, B_w_down)
    return x
```

```python
import math

import jax
import jax.numpy as jnp
from jax import lax
import jax.experimental.pallas as pl
import jax.experimental.pallas.tpu as pltpu

S, D, H, DH, F = 2048, 512, 32, 16, 1792
EPS = 1e-5
QSCALE = (DH ** -0.5) * math.log2(math.e)

TR = 256
FC = 256
TQ = 512
KC = 128
NUS = 2
NQ = S // TQ
NU = H * NQ
NC = S // KC
NS = NU // NUS
F32 = jnp.float32
BF16 = jnp.bfloat16


def _ln(x):
    mu = jnp.mean(x, axis=-1, keepdims=True)
    xc = x - mu
    var = jnp.mean(xc * xc, axis=-1, keepdims=True)
    return xc * lax.rsqrt(var + EPS)


def _kernel(x_ref, wqkv_ref, wo_ref, wg_ref, wu_ref, wd_ref, o_ref,
            xs, wqvt, kk, qm, vt, ot, hs, sa, sb, ma, mb):
    xs[...] = x_ref[...].astype(F32)
    for j in range(4):
        wqvt[j * 128:(j + 1) * 128, :] = wqkv_ref[:, j * 128:(j + 1) * 128].astype(F32).T.astype(BF16)
        wqvt[D + j * 128:D + (j + 1) * 128, :] = (
            wqkv_ref[:, 2 * D + j * 128:2 * D + (j + 1) * 128].astype(F32).T.astype(BF16))
    qm[...] = jnp.zeros(qm.shape, qm.dtype)

    def qkv_tile(r, carry):
        r0 = pl.multiple_of(r * TR, TR)
        xn = _ln(xs[pl.ds(r0, TR), :]).astype(BF16)
        k = jnp.dot(xn, wqkv_ref[:, D:2 * D], preferred_element_type=F32).astype(BF16)
        for g in range(4):
            kk[g, pl.ds(r0, TR), :] = k[:, g * 128:(g + 1) * 128]
        qv = lax.dot_general(wqvt[...], xn, (((1,), (1,)), ((), ())), preferred_element_type=F32)
        q = (qv[:D] * QSCALE).astype(BF16)
        for h in range(H):
            qm[h, (h % 8) * DH:(h % 8 + 1) * DH, pl.ds(r0, TR)] = q[h * DH:(h + 1) * DH]
        vt[:, pl.ds(r0, TR)] = qv[D:].astype(BF16)
        return carry

    def idx(u):
        h = u // NQ
        q0 = pl.multiple_of((u % NQ) * TQ, TQ)
        return h, q0, h // 8, pl.multiple_of(h * DH, DH)

    def attn_step(st_next, st_cur, s_next, s_cur, m_next, m_cur, do_cur=True):
        state = {}

        def qk(j, c):
            hn, qn, gn, _ = idx(st_next * NUS + j)
            if c == 0:
                state["mx"] = jnp.full((8, TQ), -jnp.inf, F32)
            w = qm[hn, :, pl.ds(qn, TQ)]
            s = jnp.dot(kk[gn, pl.ds(c * KC, KC), :], w, preferred_element_type=F32)
            s_next[j, pl.ds(c * KC, KC), :] = s
            mx = state["mx"]
            for i in range(KC // 8):
                mx = jnp.maximum(mx, s[i * 8:(i + 1) * 8])
            state["mx"] = mx
            if c == NC - 1:
                m_next[j] = jnp.max(mx, axis=0, keepdims=True)

        def pv(j, c):
            _, qc, _, rc = idx(st_cur * NUS + j)
            if c == 0:
                state["l"] = jnp.zeros((8, TQ), F32)
                state["acc"] = jnp.zeros((DH, TQ), F32)
                state["m"] = m_cur[j]
            p = jnp.exp2(s_cur[j, pl.ds(c * KC, KC), :] - state["m"])
            l = state["l"]
            for t in range(KC // 128):
                for i in reversed(range(16)):
                    r = t * 128 + i * 8
                    l = l + p[r:r + 8]
            state["l"] = l
            state["acc"] = state["acc"] + jnp.dot(
                vt[pl.ds(rc, DH), pl.ds(c * KC, KC)], p.astype(BF16), preferred_element_type=F32)
            if c == NC - 1:
                lt = jnp.sum(l, axis=0, keepdims=True)
                ot[pl.ds(rc, DH), pl.ds(qc, TQ)] = (state["acc"] * (1.0 / lt)).astype(BF16)

        for j in range(NUS):
            for c in range(NC):
                qk(j, c)
                if do_cur:
                    pv(j, c)

    def attn_body(i, carry):
        @pl.when(i % 2 == 0)
        def _():
            attn_step(i + 1, i, sb, sa, mb, ma)

        @pl.when(i % 2 == 1)
        def _():
            attn_step(jnp.minimum(i + 1, NS - 1), i, sa, sb, ma, mb)
        return carry

    def ffn_tile(r, carry):
        r0 = pl.multiple_of(r * TR, TR)
        o = ot[:, pl.ds(r0, TR)].astype(F32).T.astype(BF16)
        x1 = xs[pl.ds(r0, TR), :] + jnp.dot(o, wo_ref[...], preferred_element_type=F32)
        xn = _ln(x1).astype(BF16)
        for c in range(F // FC):
            g = jnp.dot(xn, wg_ref[:, c * FC:(c + 1) * FC], preferred_element_type=F32)
            u = jnp.dot(xn, wu_ref[:, c * FC:(c + 1) * FC], preferred_element_type=F32)
            hs[:, c * FC:(c + 1) * FC] = (g * u).astype(BF16)
        xs[pl.ds(r0, TR), :] = x1 + jnp.dot(hs[...], wd_ref[...], preferred_element_type=F32)
        return carry

    def layer(_, carry):
        lax.fori_loop(0, S // TR, qkv_tile, 0)
        attn_step(0, None, sa, None, ma, None, do_cur=False)
        lax.fori_loop(0, NS, attn_body, 0)
        lax.fori_loop(0, S // TR, ffn_tile, 0)
        return carry

    lax.fori_loop(0, 2, layer, 0)
    o_ref[...] = xs[...].astype(o_ref.dtype)


@jax.jit
def pallas_interleave_layers__softmax_full_mha__glu_gated_bilinear__prompt_kernel(
    A_x: jax.Array,
    A_wqkv: jax.Array,
    A_wo: jax.Array,
    B_x: jax.Array,
    B_w_gate: jax.Array,
    B_w_up: jax.Array,
    B_w_down: jax.Array,
):
    del B_x
    x = A_x.reshape(S, D)
    out = pl.pallas_call(
        _kernel,
        out_shape=jax.ShapeDtypeStruct((S, D), A_x.dtype),
        scratch_shapes=[
            pltpu.VMEM((S, D), F32),
            pltpu.VMEM((2 * D, D), BF16),
            pltpu.VMEM((4, S, 128), BF16),
            pltpu.VMEM((H, 128, S), BF16),
            pltpu.VMEM((D, S), BF16),
            pltpu.VMEM((D, S), BF16),
            pltpu.VMEM((TR, F), BF16),
            pltpu.VMEM((NUS, S, TQ), F32),
            pltpu.VMEM((NUS, S, TQ), F32),
            pltpu.VMEM((NUS, 1, TQ), F32),
            pltpu.VMEM((NUS, 1, TQ), F32),
        ],
        compiler_params=pltpu.CompilerParams(vmem_limit_bytes=100 * 1024 * 1024),
    )(x, A_wqkv, A_wo, B_w_gate, B_w_up, B_w_down)
    return out.reshape(1, S, D)
```

```python
import functools
import math

import jax
import jax.numpy as jnp
from jax import lax
import jax.experimental.pallas as pl
import jax.experimental.pallas.tpu as pltpu

S, D, H, DH, F = 2048, 512, 32, 16, 1792
EPS = 1e-5
QSCALE = (DH ** -0.5) * math.log2(math.e)

TB = 256
TS = 128
NSUB = TB // TS
NB = S // TB
FC = 256
TQ = 512
NQ = S // TQ
NCOL = TQ // 128
NC = S // 128
TIE = 0
OFF = 2
KR0 = 0
KB0 = KR0 + S // 2
QE0 = KB0 + NC * DH * 16
ZR0 = QE0 + NC * DH * 8
HB_ROWS = ZR0 + 32
L_LO = 2.0 ** -20
L_HI = 2.0 ** 60
F32 = jnp.float32
BF16 = jnp.bfloat16
U32 = jnp.uint32


def _ln(x):
    mu = jnp.mean(x, axis=-1, keepdims=True)
    xc = x - mu
    var = jnp.mean(xc * xc, axis=-1, keepdims=True)
    return (xc * lax.rsqrt(var + EPS)).astype(BF16)


def _rev_blocks(a):
    return jnp.concatenate([a[(7 - i) * 16:(8 - i) * 16] for i in range(8)], axis=0)


def _kernel(x_hbm, wqkv_hbm, wo_hbm, wg_hbm, wu_hbm, wd_hbm, o_hbm,
            xin, wqkv, wo, wg, wu, wd, xs, wqvt, kk, qt, vt, ot, hs, zer,
            hba, hbb, bad, sbuf, zs,
            sem_x, sem_w, sem_o):
    def x_copy(b):
        return pltpu.make_async_copy(x_hbm.at[pl.ds(b * TB, TB)], xin.at[pl.ds(b * TB, TB)], sem_x.at[b])

    def o_copy(b):
        return pltpu.make_async_copy(xin.at[pl.ds(b * TB, TB)], o_hbm.at[pl.ds(b * TB, TB)], sem_o.at[b])

    w_copies = [pltpu.make_async_copy(src, dst, sem_w.at[i]) for i, (src, dst) in enumerate(
        [(wqkv_hbm, wqkv), (wo_hbm, wo), (wg_hbm, wg), (wu_hbm, wu), (wd_hbm, wd)])]
    w_copies[0].start()
    x_copy(0).start()
    zer[...] = jnp.zeros(zer.shape, zer.dtype)
    for n in range(NCOL + 1):
        zs[n] = 0
    hba[ZR0:ZR0 + 8, :] = jnp.zeros((8, 128), F32)
    hbb[ZR0:ZR0 + 8, :] = jnp.zeros((8, 128), F32)
    w_copies[0].wait()
    for b in range(1, NB):
        x_copy(b).start()
    for j in range(4):
        wqvt[j * 128:(j + 1) * 128, :] = wqkv[:, j * 128:(j + 1) * 128].astype(F32).T.astype(BF16)
        wqvt[D + j * 128:D + (j + 1) * 128, :] = (
            wqkv[:, 2 * D + j * 128:2 * D + (j + 1) * 128].astype(F32).T.astype(BF16))

    def qkv(xn, t):
        r0 = pl.multiple_of(t * TS, TS)
        p0 = pl.multiple_of(t * (TS // 2), TS // 2)
        k = _rev_blocks(jnp.dot(xn, wqkv[:, D:2 * D], preferred_element_type=F32)).astype(BF16)
        for g in range(4):
            kp = pltpu.bitcast(k[:, g * 128:(g + 1) * 128], F32)
            kk[g, pl.ds(p0, TS // 2), :] = kp
            if g == 0:
                hba[pl.ds(KR0 + p0, TS // 2), :] = kp
        k16 = k[0:16, 0:128].astype(F32)
        kb0 = pl.multiple_of(KB0 + t * (DH * 16), 16)
        for d in range(DH):
            hba[pl.ds(kb0 + d * 16, 16), :] = jnp.broadcast_to(k16[:, d:d + 1], (16, 128))
        qv = lax.dot_general(wqvt[...], xn, (((1,), (1,)), ((), ())), preferred_element_type=F32)
        q = (qv[:D] * QSCALE).astype(BF16)
        qt[:, pl.ds(r0, TS)] = q
        vt[:, pl.ds(r0, TS)] = qv[D:].astype(BF16)
        q0 = q[0:DH].astype(F32)
        qe0 = pl.multiple_of(QE0 + t * (DH * 8), 8)
        for d in range(DH):
            hba[pl.ds(qe0 + d * 8, 8), :] = jnp.broadcast_to(q0[d:d + 1], (8, TS))

    def qkv_block(b, carry):
        x_copy(b).wait()
        for s in range(NSUB):
            t = b * NSUB + s
            qkv(_ln(xin[pl.ds(pl.multiple_of(t * TS, TS), TS), :].astype(F32)), t)
        return carry

    def prep_piece(h, hb, k):
        g = lax.shift_right_logical(h, 3)
        lane0 = (h & 7) * DH
        r0 = pl.multiple_of(h * DH, DH)
        rot = (lax.broadcasted_iota(jnp.int32, (8, 128), 1) + lane0) & 127
        for row in (k * 16, k * 16 + 8):
            hb[KR0 + row:KR0 + row + 8, :] = jnp.take_along_axis(
                kk[g, row:row + 8, :], rot, axis=1, mode="promise_in_bounds")
        d, i = divmod(k, 4)
        idx = jnp.full((8, 128), lane0 + d, jnp.int32)
        for t in range(4 * i, 4 * i + 4):
            col = jnp.take_along_axis(kk[g, t * 64:t * 64 + 8, :], idx, axis=1, mode="promise_in_bounds")
            kb = KB0 + (t * DH + d) * 16
            hb[kb:kb + 16, :] = pltpu.bitcast(col, BF16).astype(F32)
        t, i = divmod(k, 4)
        q = qt[pl.ds(r0, DH), t * 128:(t + 1) * 128].astype(F32)
        for d in range(4 * i, 4 * i + 4):
            qe = QE0 + (t * DH + d) * 8
            hb[qe:qe + 8, :] = jnp.broadcast_to(q[d:d + 1, :], (8, 128))

    def fast_step(h, hb, hn, hb_next):
        r0 = pl.multiple_of(h * DH, DH)
        T = NQ * NC
        pblk, lsum, acc = {}, {}, {}
        zz = [pl.multiple_of(zs[n] * 256, 256) for n in range(NCOL + 1)]

        def ladd(j, n, p8):
            l = lsum.get((j, n))
            if l is None:
                l = zer[0:8, 0:128]
            lsum[(j, n)] = l + p8

        def vpu_part(t, n):
            j, c = divmod(t, NC)
            sv = [None, None]
            for d in range(DH):
                qe = QE0 + ((j * NCOL + n) * DH + d) * 8
                q8 = hb[qe:qe + 8, :]
                for x in range(2):
                    tt = hb[pl.ds(KB0 + (c * DH + d) * 16 + x * 8 + zz[n], 8), :] * q8
                    sv[x] = tt if sv[x] is None else sv[x] + tt
            for x in range(2):
                p = jnp.exp2(sv[x])
                ladd(j, n, p)
                pblk[(j, c, 0, n, x)] = p
                if c == 0 and j > 0 and not done.get((j - 1, n)):
                    lsum[(j - 1, n)] = jnp.where(p < 0.0, p, lsum[(j - 1, n)])

        done = {}

        def dot_blocks(j, blist, vsched):
            if not blist:
                return
            w = jnp.concatenate(
                [qt[pl.ds(r0, DH), j * TQ:(j + 1) * TQ], jnp.zeros((128 - DH, TQ), BF16)], axis=0)
            kc = pltpu.bitcast(
                jnp.concatenate([hb[KR0 + c * 64 + b * 8:KR0 + c * 64 + b * 8 + 8, :] for (c, b) in blist],
                                axis=0), BF16)
            s = jnp.dot(kc, w, preferred_element_type=F32)
            for i, (c, b) in enumerate(blist):
                for f in vsched.pop(0):
                    f()
                p = jnp.exp2(s[i * 16:(i + 1) * 16])
                for n in range(NCOL):
                    for x in range(2):
                        p8 = p[x * 8:(x + 1) * 8, n * 128:(n + 1) * 128]
                        ladd(j, n, p8)
                        pblk[(j, c, b, n, x)] = p8
                    if c == NC - 1 and b == 7:
                        done[(j, n)] = True

        def qk(t):
            j0, l0, j1, l1 = None, [], None, []
            if 1 <= t <= T:
                j0, c0 = divmod(t - 1, NC)
                l0 = [(c0, b) for b in range(1 + OFF, 8)]
            if t < T:
                j1, c1 = divmod(t, NC)
                l1 = [(c1, b) for b in range(1, 1 + OFF)]
            nb = len(l0) + len(l1)
            vs = [[] for _ in range(max(nb, 1))]
            if t < T:
                for n in range(NCOL):
                    pos = min((n * 7) // NCOL + 1, nb - 1) if nb == 7 else 0
                    vs[pos].append(functools.partial(vpu_part, t, n))
            if j0 == j1:
                dot_blocks(j0, l0 + l1, vs)
            else:
                dot_blocks(j0, l0, vs)
                dot_blocks(j1, l1, vs)

        def pv(t):
            j, c = divmod(t, NC)
            pt = jnp.concatenate([
                jnp.concatenate([pblk.pop((j, c, b, n, x)) for n in range(NCOL)], axis=1)
                for b in reversed(range(8)) for x in range(2)], axis=0).astype(BF16)
            a = acc.get(j)
            if a is None:
                a = zer[...]
            a = a + jnp.dot(vt[pl.ds(r0, DH), c * 128:(c + 1) * 128], pt, preferred_element_type=F32)
            acc[j] = a
            if c == NC - 1:
                lt = jnp.sum(jnp.concatenate([lsum[(j, n)] for n in range(NCOL)], axis=1),
                             axis=0, keepdims=True)
                o = a * (1.0 / lt)
                ot[pl.ds(r0, DH), j * TQ:(j + 1) * TQ] = o.astype(BF16)
                ok = (jnp.abs(o) < 1e38) & (lt >= L_LO) & (lt <= L_HI)
                bad[...] = jnp.maximum(bad[...], jnp.where(ok, 0.0, 1.0))

        ties = []
        for t in range(T + 2):
            if TIE and len(ties) >= TIE and t - 1 < T:
                ladd((t - 1) // NC, t % NCOL, ties.pop(0))
            qk(t)
            if t >= 2:
                pv(t - 2)
            if t < T:
                prep_piece(hn, hb_next, t)
                if TIE:
                    ties.append(hb_next[pl.ds(ZR0 + zz[NCOL], 8), :])

    def fast_body(h, carry):
        hn = jnp.minimum(h + 1, H - 1)

        @pl.when(h % 2 == 0)
        def _():
            with jax.named_scope('stepA'):
                fast_step(h, hba, hn, hbb)

        @pl.when(h % 2 == 1)
        def _():
            with jax.named_scope('stepB'):
                fast_step(h, hbb, hn, hba)
        return carry

    def safe_unit(u, carry):
        h = lax.shift_right_logical(u, 2)
        g = lax.shift_right_logical(h, 3)
        q0 = pl.multiple_of((u & (NQ - 1)) * TQ, TQ)
        r0 = pl.multiple_of(h * DH, DH)
        rows = lax.broadcasted_iota(jnp.int32, (128, TQ), 0)
        qg = qt[pl.ds(pl.multiple_of(g * 128, 128), 128), pl.ds(q0, TQ)].astype(F32)
        w = jnp.where(lax.shift_right_logical(rows, 4) == (h & 7), qg, 0.0).astype(BF16)

        def scores(c, m):
            kc = pltpu.bitcast(kk[g, pl.ds(pl.multiple_of(c * 64, 64), 64), :], BF16)
            s = _rev_blocks(jnp.dot(kc, w, preferred_element_type=F32))
            sbuf[pl.ds(pl.multiple_of(c * 128, 128), 128), :] = s
            return jnp.maximum(m, jnp.max(s, axis=0, keepdims=True))

        m = lax.fori_loop(0, NC, scores, jnp.full((1, TQ), -jnp.inf, F32))

        def weigh(c, la):
            l, a = la
            c0 = pl.multiple_of(c * 128, 128)
            p = jnp.exp2(sbuf[pl.ds(c0, 128), :] - m)
            l = l + jnp.sum(p, axis=0, keepdims=True)
            a = a + jnp.dot(vt[pl.ds(r0, DH), pl.ds(c0, 128)], p.astype(BF16), preferred_element_type=F32)
            return l, a

        l, a = lax.fori_loop(0, NC, weigh, (jnp.zeros((1, TQ), F32), jnp.zeros((DH, TQ), F32)))
        ot[pl.ds(r0, DH), pl.ds(q0, TQ)] = (a * (1.0 / l)).astype(BF16)
        return carry

    def ffn_block(b, first):
        r0 = [pl.multiple_of(b * TB + s * TS, TS) for s in range(NSUB)]
        x1 = []
        for s in range(NSUB):
            o = ot[:, pl.ds(r0[s], TS)].astype(F32).T.astype(BF16)
            res = xin[pl.ds(r0[s], TS), :].astype(F32) if first else xs[pl.ds(r0[s], TS), :]
            x1.append(res + jnp.dot(o, wo[...], preferred_element_type=F32))
        x2 = []
        for s in range(NSUB):
            xn = _ln(x1[s])
            for c in range(F // FC):
                g = jnp.dot(xn, wg[:, c * FC:(c + 1) * FC], preferred_element_type=F32)
                u = jnp.dot(xn, wu[:, c * FC:(c + 1) * FC], preferred_element_type=F32)
                hs[s, :, c * FC:(c + 1) * FC] = (g * u).astype(BF16)
            x2.append(x1[s] + jnp.dot(hs[s], wd[...], preferred_element_type=F32))
            if first:
                xs[pl.ds(r0[s], TS), :] = x2[s]
            else:
                xin[pl.ds(r0[s], TS), :] = x2[s].astype(BF16)
        if first:
            for s in range(NSUB):
                qkv(_ln(x2[s]), b * NSUB + s)
        else:
            o_copy(b).start()

    def ffn_first(b, carry):
        ffn_block(b, True)
        return carry

    def ffn_last(b, carry):
        ffn_block(b, False)
        return carry

    with jax.named_scope("phaseA"):
        lax.fori_loop(0, NB, qkv_block, 0)
    for cp in w_copies[1:]:
        cp.start()

    def layer(li, carry):
        bad[...] = jnp.zeros(bad.shape, bad.dtype)
        with jax.named_scope("attn"):
            lax.fori_loop(0, H, fast_body, 0)

        @pl.when(jnp.max(bad[...]) > 0.0)
        def _():
            lax.fori_loop(0, H * NQ, safe_unit, 0)

        @pl.when(li == 0)
        def _():
            for cp in w_copies[1:]:
                cp.wait()
            with jax.named_scope("ffn_first"):
                lax.fori_loop(0, NB, ffn_first, 0)

        @pl.when(li == 1)
        def _():
            with jax.named_scope("ffn_last"):
                lax.fori_loop(0, NB, ffn_last, 0)
        return carry

    lax.fori_loop(0, 2, layer, 0)
    for b in range(NB):
        o_copy(b).wait()


@jax.jit
def pallas_interleave_layers__softmax_full_mha__glu_gated_bilinear__prompt_kernel(
    A_x: jax.Array,
    A_wqkv: jax.Array,
    A_wo: jax.Array,
    B_x: jax.Array,
    B_w_gate: jax.Array,
    B_w_up: jax.Array,
    B_w_down: jax.Array,
):
    del B_x
    x = A_x.reshape(S, D)
    any_spec = pl.BlockSpec(memory_space=pl.ANY)
    out = pl.pallas_call(
        _kernel,
        out_shape=jax.ShapeDtypeStruct((S, D), A_x.dtype),
        in_specs=[any_spec] * 6,
        out_specs=any_spec,
        scratch_shapes=[
            pltpu.VMEM((S, D), BF16),
            pltpu.VMEM((D, 3 * D), BF16),
            pltpu.VMEM((D, D), BF16),
            pltpu.VMEM((D, F), BF16),
            pltpu.VMEM((D, F), BF16),
            pltpu.VMEM((F, D), BF16),
            pltpu.VMEM((S, D), F32),
            pltpu.VMEM((2 * D, D), BF16),
            pltpu.VMEM((4, S // 2, 128), F32),
            pltpu.VMEM((D, S), BF16),
            pltpu.VMEM((D, S), BF16),
            pltpu.VMEM((D, S), BF16),
            pltpu.VMEM((NSUB, TS, F), BF16),
            pltpu.VMEM((DH, TQ), F32),
            pltpu.VMEM((HB_ROWS, 128), F32),
            pltpu.VMEM((HB_ROWS, 128), F32),
            pltpu.VMEM((DH, TQ), F32),
            pltpu.VMEM((S, TQ), F32),
            pltpu.SMEM((NCOL + 1,), jnp.int32),
            pltpu.SemaphoreType.DMA((NB,)),
            pltpu.SemaphoreType.DMA((5,)),
            pltpu.SemaphoreType.DMA((NB,)),
        ],
        compiler_params=pltpu.CompilerParams(vmem_limit_bytes=100 * 1024 * 1024),
    )(x, A_wqkv, A_wo, B_w_gate, B_w_up, B_w_down)
    return out.reshape(1, S, D)
```

```python
import functools
import math

import jax
import jax.numpy as jnp
from jax import lax
import jax.experimental.pallas as pl
import jax.experimental.pallas.tpu as pltpu

S, D, H, DH, F = 2048, 512, 32, 16, 1792
EPS = 1e-5
QSCALE = (DH ** -0.5) * math.log2(math.e)

TB = 256
TS = 128
NSUB = TB // TS
NB = S // TB
HD = D // 2
HF = F // 2
NF = HF // 128
NSC = NF // 2
GU_EARLY = ((0, 0), (0, 1))
SC_ORDER = (0, 1, 2, 3)
OTIE = 3
IN_ORDER = (0, 3, 4, 6, 2, 1, 5)
GU_ORDER = (2, 4, 0, 3, 6, 1, 5)
DN_ORDER = (0, 3, 4, 6, 2, 1, 5)
TQ = 512
NQ = S // TQ
NCOL = TQ // 128
NC = S // 128
T = NQ * NC
OFF = 2
VPOS = (1, 2, 4, 6)
NH = 2
TT = NH * T
XGAPS = (3, 3, 3, 3, 4)
XPOS = (3, 5)
XSH = 2
PPP = 2
ALAG = 2
DG = 4
DCH = 1

NV = [1] * TT
XS = [[] for _ in range(TT + 1)]
_prev = XSH - 1
for _gap in XGAPS * (TT // sum(XGAPS)):
    _t = _prev + _gap
    if _t >= TT - 1:
        break
    NV[_t] += 1
    for _n in range(NCOL):
        for _x in range(2):
            XS[_prev + 1 + ((2 * _n + _x) * _gap) // (2 * NCOL)].append((_t, _n, NV[_t] - 1, XPOS[_x], (_x,)))
    _prev = _t
NVC = [max(NV[c::NC]) for c in range(NC)]
NVMAX = max(NVC)

KR0 = 0
KB0 = KR0 + S // 2
HB_ROWS = KB0 + NC * NVMAX * DH * 16
L_LO = 2.0 ** -40
L_HI = 2.0 ** 60
F32 = jnp.float32
BF16 = jnp.bfloat16


def _ln(x):
    mu = jnp.mean(x, axis=-1, keepdims=True)
    xc = x - mu
    var = jnp.mean(xc * xc, axis=-1, keepdims=True)
    return xc * lax.rsqrt(var + EPS)


def _pk(a):
    return pltpu.bitcast(a, F32)


def _up(a):
    return pltpu.bitcast(a, BF16)


def _mm(a, b):
    return lax.dot_general(a, b, (((1,), (0,)), ((), ())), preferred_element_type=F32)


def _lhs7(a11, a12, a21, a22):
    return [a11 + a22, a21 + a22, a11, a22, a11 + a12, a21 - a11, a12 - a22]


def _rhs7(b11, b12, b21, b22):
    return [b11 + b22, b11, b12 - b22, b21 - b11, b22, b11 + b12, b21 + b22]


def _quads(a):
    r, c = a.shape[0] // 2, a.shape[1] // 2
    return a[:r, :c], a[:r, c:], a[r:, :c], a[r:, c:]


def _combine7(m):
    return (m[0] + m[3] - m[4] + m[6], m[2] + m[4], m[1] + m[3], m[0] - m[1] + m[2] + m[5])


def _rev_blocks(a):
    return jnp.concatenate([a[(15 - i) * 8:(16 - i) * 8] for i in range(16)], axis=0)


def _mult(v, m):
    return v if isinstance(v, int) else pl.multiple_of(v, m)


def _kernel(x_hbm, wqkv_hbm, wo_hbm, wg_hbm, wu_hbm, wd_hbm, o_hbm,
            xin, wqkv, wo, wg, wu, wd, wgu1, wgu2, wdn, xs, wqvt, kk, kv, qt, vt, ot, on, hs, zer,
            hba, hbb, qe, lt, chk, pc, ac, lc, sbuf, vsum, zs,
            sem_x, sem_w, sem_o):
    def x_copy(b):
        return pltpu.make_async_copy(x_hbm.at[pl.ds(b * TB, TB)], xin.at[pl.ds(b * TB, TB)], sem_x.at[b])

    def o_copy(b):
        return pltpu.make_async_copy(xin.at[pl.ds(b * TB, TB)], o_hbm.at[pl.ds(b * TB, TB)], sem_o.at[b])

    w_copies = [pltpu.make_async_copy(src, dst, sem_w.at[i]) for i, (src, dst) in enumerate(
        [(wo_hbm, wo), (wg_hbm, wg), (wu_hbm, wu), (wd_hbm, wd)])]
    qkv_copies = [pltpu.make_async_copy(wqkv_hbm.at[:, pl.ds(i * D, D)], wqkv.at[:, pl.ds(i * D, D)],
                                        sem_w.at[4 + i]) for i in range(3)]

    def k_proj(xn, t):
        p0 = _mult(t * (TS // 2), TS // 2)
        k = _rev_blocks(jnp.dot(xn, wqkv[:, D:2 * D], preferred_element_type=F32)).astype(BF16)
        kf = k[0:NVMAX * 16].astype(F32)
        for g in range(4):
            kp = _pk(k[:, g * 128:(g + 1) * 128])
            kk[g, pl.ds(p0, TS // 2), :] = kp
            kv[g, pl.ds(_mult(t * (NVMAX * 16), 16), NVMAX * 16), :] = kf[:, g * 128:(g + 1) * 128]
            if g == 0:
                hba[pl.ds(KR0 + p0, TS // 2), :] = kp
        for b in range(NVMAX):
            kb0 = _mult(KB0 + (t * NVMAX + b) * (DH * 16), 16)
            for d in range(DH):
                hba[pl.ds(kb0 + d * 16, 16), :] = jnp.broadcast_to(kf[b * 16:(b + 1) * 16, d:d + 1], (16, 128))

    def nt(w, xn):
        return lax.dot_general(_up(w), xn, (((1,), (1,)), ((), ())), preferred_element_type=F32)

    def q_store(qf, t):
        q = (qf * QSCALE).astype(BF16)
        qt[:, pl.ds(_mult(t * TS, TS), TS)] = _pk(q)
        qe[:, pl.ds(_mult(t * (DH * 8), DH * 8), DH * 8), :] = jnp.broadcast_to(
            q.astype(F32)[:, None, :], (D, 8, TS)).reshape(H, DH * 8, TS)

    def v_store(v, t):
        vt[:, pl.ds(_mult(t * TS, TS), TS)] = _pk(v.astype(BF16))
        vsum[...] = vsum[...] + jnp.sum(jnp.abs(v).reshape(D // 8, 8, TS), axis=0)

    def qv_proj(xn, t):
        qv = nt(wqvt[...], xn)
        q_store(qv[:D], t)
        v_store(qv[D:], t)

    def ln_in(b):
        for s in range(NSUB):
            r0 = _mult(b * TB + s * TS, TS)
            on[s] = _pk(_ln(xin[pl.ds(r0, TS), :].astype(F32)).astype(BF16))

    def qkv_block(b, carry):
        nxt = jnp.minimum(b + 1, NB - 1)

        @pl.when(b + 1 < NB)
        def _():
            x_copy(b + 1).wait()
        for s in range(NSUB):
            k_proj(_up(on[s]), b * NSUB + s)
            qv_proj(_up(on[s]), b * NSUB + s)
        ln_in(nxt)
        return carry

    def prep_piece(h, hb, k):
        g = lax.shift_right_logical(h, 3)
        lane0 = (h & 7) * DH
        rot = (lax.broadcasted_iota(jnp.int32, (8, 128), 1) + lane0) & 127
        for row in (k * 16, k * 16 + 8):
            hb[KR0 + row:KR0 + row + 8, :] = jnp.take_along_axis(
                kk[g, row:row + 8, :], rot, axis=1, mode="promise_in_bounds")
        d, i = divmod(k, 4)
        idx = jnp.full((8, 128), lane0 + d, jnp.int32)
        for c in range(4 * i, 4 * i + 4):
            for b in range(NVC[c]):
                for x in range(2):
                    src = (c * NVMAX + b) * 16 + x * 8
                    dst = KB0 + ((c * NVMAX + b) * DH + d) * 16 + x * 8
                    hb[dst:dst + 8, :] = jnp.take_along_axis(
                        kv[g, src:src + 8, :], idx, axis=1, mode="promise_in_bounds")

    def finish(h, j, a, l8):
        ot[pl.ds(_mult(h * DH, DH), DH), j * TQ:(j + 1) * TQ] = a
        for n in range(NCOL):
            lt[j * NCOL + n, pl.ds(_mult(h * 8, 8), 8), :] = l8[:, n * 128:(n + 1) * 128]
        chk[0] = chk[0] + l8
        chk[1] = jnp.minimum(chk[1], l8)

    def flush(h):
        a = ac[...] + _mm(_up(vt[pl.ds(_mult(h * 8, 8), 8), S - 128:S]), pc[...])
        finish(h, NQ - 1, a, lc[...])

    def fast_step(i, carry):
        hs_ = [NH * i + k for k in range(NH)]
        hbs = (hba, hbb)
        r0 = [pl.multiple_of(h * 8, 8) for h in hs_]
        pblk, lsum, acc, done, snap = {}, {}, {}, {}, {}
        zz = [pl.multiple_of(zs[n] * 256, 256) for n in range(NCOL + 2)]

        def ladd(u, n, p8):
            l = lsum.get((u, n))
            if l is None:
                l = zer[0:8, 0:128]
            lsum[(u, n)] = l + p8

        def vpu_part(t, n, b, xs_):
            u, c = divmod(t, NC)
            hb = hbs[t // T]
            sv = None
            for d0 in range(0, DH, DG):
                row = (((u % NQ) * NCOL + n) * DH + d0) * 8
                q8 = (qe[hs_[t // T], pl.ds(row + zz[NCOL + 1], DG * 8), :] if b
                      else qe[hs_[t // T], row:row + DG * 8, :]).reshape(DG, 1, 8, 128)
                if t == TT - 1:
                    q8 = jnp.where(snap[n] < 0.0, 0.0, q8)
                kb = hb[pl.ds(KB0 + ((c * NVMAX + b) * DH + d0) * 16 + zz[n], DG * 16), :].reshape(DG, 2, 8, 128)
                if len(xs_) == 1:
                    kb = kb[:, xs_[0]:xs_[0] + 1]
                pr = kb * q8
                if DCH:
                    if sv is not None:
                        pr = jnp.concatenate([sv[None], pr], axis=0)
                    sv = jnp.sum(pr, axis=0)
                else:
                    pr = jnp.sum(pr, axis=0)
                    sv = pr if sv is None else sv + pr
            sv = {x: sv[m] for m, x in enumerate(xs_)}
            for x in xs_:
                p = jnp.exp2(sv[x])
                ladd(u, n, p)
                if t == TT - ALAG:
                    snap[n] = lsum[(u, n)]
                pblk[(t, b, n, x)] = p
                if u > 0 and not done.get((u - 1, n)):
                    lsum[(u - 1, n)] = jnp.where(p < 0.0, p, lsum[(u - 1, n)])

        def dot_blocks(blist, vsched):
            if not blist:
                return
            u = blist[0][0] // NC
            k, j = divmod(u, NQ)
            w = jnp.concatenate(
                [_up(qt[pl.ds(r0[k], 8), j * TQ:(j + 1) * TQ]), jnp.zeros((128 - DH, TQ), BF16)], axis=0)
            kc = _up(jnp.concatenate(
                [hbs[k][pl.ds(KR0 + (t % NC) * 64 + b * 8 + zz[NCOL], 8), :] for (t, b) in blist], axis=0))
            s = jnp.dot(kc, w, preferred_element_type=F32)
            for m, (t, b) in enumerate(blist):
                for f in vsched.pop(0):
                    f()
                p = jnp.exp2(s[m * 16:(m + 1) * 16])
                for n in range(NCOL):
                    for x in range(2):
                        p8 = p[x * 8:(x + 1) * 8, n * 128:(n + 1) * 128]
                        ladd(u, n, p8)
                        pblk[(t, b, n, x)] = p8
                    if t % NC == NC - 1 and b == 7:
                        done[(u, n)] = True

        def qk(t):
            l0 = [(t - 1, b) for b in range(NV[t - 1] + OFF, 8)] if t >= 1 else []
            l1 = [(t, b) for b in range(NV[t], NV[t] + OFF)] if t < TT else []
            nb = len(l0) + len(l1)
            vs = [[] for _ in range(nb)]
            parts = [(t, n, 0, VPOS[n], (0, 1)) for n in range(NCOL)] if t < TT else []
            for (tt, n, b, pos, xs_) in parts + XS[t]:
                vs[min(pos, nb - 1)].append(functools.partial(vpu_part, tt, n, b, xs_))
            if t % NC:
                dot_blocks(l0 + l1, vs)
            else:
                dot_blocks(l0, vs)
                dot_blocks(l1, vs)

        def ptile(t):
            return jnp.concatenate([
                jnp.concatenate([pblk.pop((t, b, n, x)) for n in range(NCOL)], axis=1)
                for b in reversed(range(8)) for x in (1, 0)], axis=0)

        def lrow(u):
            return jnp.concatenate([lsum[(u, n)] for n in range(NCOL)], axis=1)

        def pv(t):
            u, c = divmod(t, NC)
            k, j = divmod(u, NQ)
            a = acc.get(u)
            if a is None:
                a = zer[...]
            a = a + _mm(_up(vt[pl.ds(r0[k], 8), c * 128:(c + 1) * 128]), ptile(t))
            acc[u] = a
            if c == NC - 1:
                finish(hs_[k], j, a, lrow(u))

        for t in range(TT + 1):
            qk(t)
            if t == 1:
                flush(jnp.maximum(hs_[0] - 1, 0))
            if t >= 2:
                pv(t - 2)
            k, tl = divmod(t, T)
            if k < NH and tl * PPP < T:
                hn = jnp.minimum(hs_[k] + 1, H - 1)
                hb_next = hbs[(k + 1) % 2]
                for m in range(PPP):
                    prep_piece(hn, hb_next, tl * PPP + m)
        pc[...] = ptile(TT - 1)
        ac[...] = acc[NH * NQ - 1]
        lc[...] = lrow(NH * NQ - 1)
        return carry

    def safe_unit(u, carry):
        h = lax.shift_right_logical(u, 2)
        g = lax.shift_right_logical(h, 3)
        q0 = pl.multiple_of((u & (NQ - 1)) * TQ, TQ)
        rows = lax.broadcasted_iota(jnp.int32, (128, TQ), 0)
        qg = _up(qt[pl.ds(pl.multiple_of(g * 64, 64), 64), pl.ds(q0, TQ)]).astype(F32)
        w = jnp.where(lax.shift_right_logical(rows, 4) == (h & 7), qg, 0.0).astype(BF16)

        def scores(c, m):
            kc = _up(kk[g, pl.ds(pl.multiple_of(c * 64, 64), 64), :])
            s = _rev_blocks(jnp.dot(kc, w, preferred_element_type=F32))
            sbuf[pl.ds(pl.multiple_of(c * 128, 128), 128), :] = s
            return jnp.maximum(m, jnp.max(s, axis=0, keepdims=True))

        m = lax.fori_loop(0, NC, scores, jnp.full((1, TQ), -jnp.inf, F32))

        def weigh(c, la):
            l, a = la
            c0 = pl.multiple_of(c * 128, 128)
            p = jnp.exp2(sbuf[pl.ds(c0, 128), :] - m)
            l = l + jnp.sum(p, axis=0, keepdims=True)
            a = a + _mm(_up(vt[pl.ds(pl.multiple_of(h * 8, 8), 8), pl.ds(c0, 128)]), p.astype(BF16))
            return l, a

        l, a = lax.fori_loop(0, NC, weigh, (jnp.zeros((1, TQ), F32), jnp.zeros((DH, TQ), F32)))
        ot[pl.ds(pl.multiple_of(h * DH, DH), DH), pl.ds(q0, TQ)] = a
        l8 = jnp.broadcast_to(l * 0.125, (8, TQ))
        for n in range(NCOL):
            lt[(u & (NQ - 1)) * NCOL + n, pl.ds(pl.multiple_of(h * 8, 8), 8), :] = l8[:, n * 128:(n + 1) * 128]
        return carry

    def wprep_gu(sc, k):
        w = (wg, wu)[k]
        w_ = 256 if sc < NSC else 128
        cl = slice(sc * 256, sc * 256 + w_)
        cr = slice(HF + sc * 256, HF + sc * 256 + w_)
        r7 = _rhs7(w[:HD, cl].astype(F32), w[:HD, cr].astype(F32), w[HD:, cl].astype(F32), w[HD:, cr].astype(F32))
        for i in range(7):
            if sc < NSC:
                for m, t in enumerate(_rhs7(*_quads(r7[i]))):
                    wgu2[(sc * 7 + i) * 7 + m, :, k * 128:(k + 1) * 128] = _pk(t.astype(BF16))
            else:
                wgu1[i, :, k * 128:(k + 1) * 128] = _pk(r7[i].astype(BF16))

    def wprep_dn():
        for i, t in enumerate(_rhs7(*_quads(wd[...].astype(F32)))):
            wdn[i] = _pk(t.astype(BF16))

    def o_stage(b):
        for s in range(NSUB):
            cols = pl.ds(_mult(b * TB + s * TS, TS), TS)
            ct = b * NSUB + s
            den = lt[ct, pl.ds(0, H, stride=8), :]
            for i in range(1, 8):
                den = den + lt[ct, pl.ds(i, H, stride=8), :]
            r = 1.0 / den
            o = jnp.concatenate([ot[h * DH:(h + 1) * DH, cols] * r[h:h + 1] for h in range(H)], axis=0)
            on[s] = _pk(o.T.astype(BF16))

    def ffn_block(b, first, prep=False):
        r0 = [_mult(b * TB + s * TS, TS) for s in range(NSUB)]
        x1 = []
        if prep:
            for sc in SC_ORDER:
                for k in range(2):
                    wprep_gu(sc, k)
            wprep_dn()
        for s in range(NSUB):
            res = xin[pl.ds(r0[s], TS), :].astype(F32) if first else xs[pl.ds(r0[s], TS), :]
            x1.append(res + jnp.dot(_up(on[s]), wo[...], preferred_element_type=F32))
        o_stage(min(b + 1, NB - 1) if isinstance(b, int) else jnp.minimum(b + 1, NB - 1))
        otie = on[NSUB + zs[0], 0:8, 0:128]
        xn = [_ln(x1[s]) for s in range(NSUB)]
        la = _lhs7(xn[0][:, :HD], xn[0][:, HD:], xn[1][:, :HD], xn[1][:, HD:])
        la1 = [t.astype(BF16) for t in la]
        la2 = [[t.astype(BF16) for t in _lhs7(*_quads(a_))] for a_ in la]

        def gu(i, sc, k):
            if sc == NSC:
                return _mm(la1[i], _up(wgu1[i]))
            mi = {m: _mm(la2[i][m], _up(wgu2[(sc * 7 + i) * 7 + m, :, k * 128:(k + 1) * 128])) for m in IN_ORDER}
            c = _combine7(mi)
            return jnp.concatenate([jnp.concatenate(c[:2], axis=1), jnp.concatenate(c[2:], axis=1)], axis=0)

        early = {(i, sc, k): gu(i, sc, k) for (sc, k) in GU_EARLY for i in GU_ORDER[:2]}

        def outer(sc, k):
            return _combine7({i: early[(i, sc, k)] if (i, sc, k) in early else gu(i, sc, k) for i in GU_ORDER})

        for sc in SC_ORDER:
            if sc == NSC:
                hq = [t[:, :128] * t[:, 128:] for t in outer(sc, 0)]
            else:
                hq = [g * u for g, u in zip(outer(sc, 0), outer(sc, 1))]
            for i, t in enumerate(_lhs7(*hq)):
                hs[i, :, sc * 256:sc * 256 + t.shape[1]] = t.astype(BF16)
        m = {}
        for i in DN_ORDER:
            wi = wdn[i]
            if i == DN_ORDER[OTIE]:
                w0 = pltpu.bitcast(pltpu.bitcast(wi[:8, :128], jnp.int32) | pltpu.bitcast(otie, jnp.int32), F32)
                wi = jnp.concatenate([jnp.concatenate([w0, wi[:8, 128:]], axis=1), wi[8:]], axis=0)
            m[i] = jnp.dot(hs[i], _up(wi), preferred_element_type=F32)
        c = _combine7(m)
        x2 = [x1[s] + jnp.concatenate([c[2 * s], c[2 * s + 1]], axis=1) for s in range(NSUB)]
        for s in range(NSUB):
            if first:
                xs[pl.ds(r0[s], TS), :] = x2[s]
            else:
                xin[pl.ds(r0[s], TS), :] = x2[s].astype(BF16)
        if first:
            for s in range(NSUB):
                xn2 = _ln(x2[s]).astype(BF16)
                k_proj(xn2, b * NSUB + s)
                qv_proj(xn2, b * NSUB + s)
        else:
            o_copy(b).start()

    def ffn_first(b, carry):
        ffn_block(b, True)
        return carry

    def ffn_last(b, carry):
        ffn_block(b, False)
        return carry

    def w_transpose(i):
        for j in range(4):
            c0 = 2 * i * D + j * 128
            wqvt[i * HD + j * 64:i * HD + (j + 1) * 64, :] = _pk(wqkv[:, c0:c0 + 128].astype(F32).T.astype(BF16))

    x_copy(0).start()
    qkv_copies[1].start()
    zer[...] = jnp.zeros(zer.shape, zer.dtype)
    on[NSUB, 0:8, 0:128] = jnp.zeros((8, 128), F32)
    vsum[...] = jnp.zeros(vsum.shape, vsum.dtype)
    for n in range(NCOL + 2):
        zs[n] = 0
    with jax.named_scope("phase_x0"):
        x_copy(0).wait()
    qkv_copies[0].start()
    ln_in(0)
    with jax.named_scope("phase_w1"):
        qkv_copies[1].wait()
    qkv_copies[2].start()
    x_copy(1).start()
    with jax.named_scope("phaseA0k"):
        k_proj(_up(on[0]), 0)
    with jax.named_scope("phase_w0"):
        qkv_copies[0].wait()
    with jax.named_scope("phaseA0q"):
        k_proj(_up(on[1]), 1)
        w_transpose(0)
        q_store(nt(wqvt[:HD], _up(on[0])), 0)
    with jax.named_scope("phase_w2"):
        qkv_copies[2].wait()
        x_copy(1).wait()
    for b in range(2, NB):
        x_copy(b).start()
    with jax.named_scope("phaseA0v"):
        q_store(nt(wqvt[:HD], _up(on[1])), 1)
        w_transpose(1)
        for s in range(NSUB):
            v_store(nt(wqvt[HD:], _up(on[s])), s)
        ln_in(1)
    with jax.named_scope("phaseA"):
        lax.fori_loop(1, NB, qkv_block, 0)
    for cp in w_copies:
        cp.start()

    def layer(li, carry):
        chk[0] = jnp.zeros((8, TQ), F32)
        chk[1] = jnp.ones((8, TQ), F32)
        pc[...] = jnp.zeros(pc.shape, pc.dtype)
        ac[...] = jnp.zeros(ac.shape, ac.dtype)
        lc[...] = jnp.ones(lc.shape, lc.dtype)
        with jax.named_scope("attn"):
            lax.fori_loop(0, H // NH, fast_step, 0)
        flush(H - 1)
        o_stage(0)

        ok = (chk[0] <= L_HI) & (chk[1] >= L_LO) & (jnp.concatenate([vsum[...]] * NCOL, axis=1) <= L_HI)

        @pl.when(jnp.max(jnp.where(ok, 0.0, 1.0)) > 0.0)
        def _():
            lax.fori_loop(0, H * NQ, safe_unit, 0)
            o_stage(0)

        @pl.when(li == 0)
        def _():
            for cp in w_copies:
                cp.wait()
            with jax.named_scope("ffn_first0"):
                ffn_block(0, True, prep=True)
            with jax.named_scope("ffn_first"):
                lax.fori_loop(1, NB, ffn_first, 0)

        @pl.when(li == 1)
        def _():
            with jax.named_scope("ffn_last"):
                lax.fori_loop(0, NB, ffn_last, 0)
        return carry

    lax.fori_loop(0, 2, layer, 0)
    for b in range(NB):
        o_copy(b).wait()


@jax.jit
def pallas_interleave_layers__softmax_full_mha__glu_gated_bilinear__prompt_kernel(
    A_x: jax.Array,
    A_wqkv: jax.Array,
    A_wo: jax.Array,
    B_x: jax.Array,
    B_w_gate: jax.Array,
    B_w_up: jax.Array,
    B_w_down: jax.Array,
):
    del B_x
    x = A_x.reshape(S, D)
    any_spec = pl.BlockSpec(memory_space=pl.ANY)
    out = pl.pallas_call(
        _kernel,
        out_shape=jax.ShapeDtypeStruct((S, D), A_x.dtype),
        in_specs=[any_spec] * 6,
        out_specs=any_spec,
        scratch_shapes=[
            pltpu.VMEM((S, D), BF16),
            pltpu.VMEM((D, 3 * D), BF16),
            pltpu.VMEM((D, D), BF16),
            pltpu.VMEM((D, F), BF16),
            pltpu.VMEM((D, F), BF16),
            pltpu.VMEM((F, D), BF16),
            pltpu.VMEM((7, HD // 2, 256), F32),
            pltpu.VMEM((NSC * 49, 64, 256), F32),
            pltpu.VMEM((7, HF // 2, HD), F32),
            pltpu.VMEM((S, D), F32),
            pltpu.VMEM((D, D), F32),
            pltpu.VMEM((4, S // 2, 128), F32),
            pltpu.VMEM((4, NC * NVMAX * 16, 128), F32),
            pltpu.VMEM((HD, S), F32),
            pltpu.VMEM((HD, S), F32),
            pltpu.VMEM((D, S), F32),
            pltpu.VMEM((NSUB + 1, TS // 2, D), F32),
            pltpu.VMEM((7, TS, HF), BF16),
            pltpu.VMEM((DH, TQ), F32),
            pltpu.VMEM((HB_ROWS, 128), F32),
            pltpu.VMEM((HB_ROWS, 128), F32),
            pltpu.VMEM((H, NC * DH * 8, 128), F32),
            pltpu.VMEM((NC, H * 8, 128), F32),
            pltpu.VMEM((2, 8, TQ), F32),
            pltpu.VMEM((128, TQ), F32),
            pltpu.VMEM((DH, TQ), F32),
            pltpu.VMEM((8, TQ), F32),
            pltpu.VMEM((S, TQ), F32),
            pltpu.VMEM((8, 128), F32),
            pltpu.SMEM((NCOL + 2,), jnp.int32),
            pltpu.SemaphoreType.DMA((NB,)),
            pltpu.SemaphoreType.DMA((7,)),
            pltpu.SemaphoreType.DMA((NB,)),
        ],
        compiler_params=pltpu.CompilerParams(vmem_limit_bytes=110 * 1024 * 1024),
    )(x, A_wqkv, A_wo, B_w_gate, B_w_up, B_w_down)
    return out.reshape(1, S, D)
```

```python
import functools
import math

import jax
import jax.numpy as jnp
from jax import lax
import jax.experimental.pallas as pl
import jax.experimental.pallas.tpu as pltpu

S, D, H, DH, F = 2048, 512, 32, 16, 1792
EPS = 1e-5
QSCALE = (DH ** -0.5) * math.log2(math.e)
F32 = jnp.float32
BF16 = jnp.bfloat16

TB = 256
TS = 128
NSUB = TB // TS
NB = S // TB
HD = D // 2
HF = F // 2
NSC = HF // 256
GU_EARLY = ((0, 0), (0, 1), (1, 0))
GU_ORDER = (2, 4, 0, 3, 6, 1, 5)
IN_ORDER = (0, 3, 4, 6, 2, 1, 5)

TQ = 512
NQ = S // TQ
NCOL = TQ // 128
NC = S // 128
T = NQ * NC
NH = 2
TT = NH * T
OFF = 2
VPOS = (1, 2, 4, 6)
XGAPS = (3, 3, 3, 3, 4)
XPOS = (3, 5)
XSH = 2
PPP = 2
DG = 4
L_LO = 2.0 ** -40
L_HI = 2.0 ** 60

NV = [1] * TT
XS = [[] for _ in range(TT + 1)]
_prev = XSH - 1
for _gap in XGAPS * (TT // sum(XGAPS)):
    _t = _prev + _gap
    if _t >= TT - 1:
        break
    NV[_t] += 1
    for _n in range(NCOL):
        for _x in range(2):
            XS[_prev + 1 + ((2 * _n + _x) * _gap) // (2 * NCOL)].append((_t, _n, NV[_t] - 1, XPOS[_x], (_x,)))
    _prev = _t
NVC = [max(NV[c::NC]) for c in range(NC)]
NVMAX = max(NVC)

KR0 = 0
KB0 = KR0 + S // 2
HB_ROWS = KB0 + NC * NVMAX * DH * 16


def _ln(x):
    mu = jnp.mean(x, axis=-1, keepdims=True)
    xc = x - mu
    var = jnp.mean(xc * xc, axis=-1, keepdims=True)
    return xc * lax.rsqrt(var + EPS)


def _pk(a):
    return pltpu.bitcast(a, F32)


def _up(a):
    return pltpu.bitcast(a, BF16)


def _mm(a, b):
    return lax.dot_general(a, b, (((1,), (0,)), ((), ())), preferred_element_type=F32)


def _nt(a, b):
    return lax.dot_general(a, b, (((1,), (1,)), ((), ())), preferred_element_type=F32)


def _lhs1(i, a):
    p, sign, q = ((0, 1, 3), (2, 1, 3), (0, 0, 0), (3, 0, 0), (0, 1, 1), (2, -1, 0), (1, -1, 3))[i]
    return a(p) if sign == 0 else (a(p) + a(q) if sign > 0 else a(p) - a(q))


def _rhs7(b11, b12, b21, b22):
    return [b11 + b22, b11, b12 - b22, b21 - b11, b22, b11 + b12, b21 + b22]


def _combine7(m):
    return (m[0] + m[3] - m[4] + m[6], m[2] + m[4], m[1] + m[3], m[0] - m[1] + m[2] + m[5])


def _quads(a):
    r, c = a.shape[0] // 2, a.shape[1] // 2
    return a[:r, :c], a[:r, c:], a[r:, :c], a[r:, c:]


def _join(c):
    return jnp.concatenate([jnp.concatenate(c[:2], axis=1), jnp.concatenate(c[2:], axis=1)], axis=0)


def _rev_blocks(a):
    return jnp.concatenate([a[(15 - i) * 8:(16 - i) * 8] for i in range(16)], axis=0)


def _mult(v, m):
    return v if isinstance(v, int) else pl.multiple_of(v, m)


def _kernel(x_hbm, wqkv_hbm, wo_hbm, wg_hbm, wu_hbm, wd_hbm, o_hbm,
            xin, wq, wk, wv, wo, wg, wu, wd, wkp, wop, wgu1, wgu2, wdn1, wdn2, xs, wqvt,
            kk, kv, qt, vt, ot, on, zer, hba, hbb, qe, lt, chk, pc, ac, lc, sbuf, vsum,
            hs, xb0, xb1, zs, sem_x, sem_w, sem_o):
    xb = (xb0, xb1)

    def x_copy(b):
        return pltpu.make_async_copy(x_hbm.at[pl.ds(b * TB, TB)], xin.at[pl.ds(b * TB, TB)], sem_x.at[b])

    def o_copy(b):
        return pltpu.make_async_copy(xin.at[pl.ds(b * TB, TB)], o_hbm.at[pl.ds(b * TB, TB)], sem_o.at[b])

    w_copies = [pltpu.make_async_copy(src, dst, sem_w.at[i]) for i, (src, dst) in enumerate(
        [(wo_hbm, wo), (wg_hbm, wg), (wu_hbm, wu), (wd_hbm, wd)])]
    wq_copy, wk_copy, wv_copy = [
        pltpu.make_async_copy(wqkv_hbm.at[:, pl.ds(i * D, D)], dst, sem_w.at[4 + i])
        for i, dst in enumerate((wq, wk, wv))]

    def k_proj(xn, t):
        p0 = _mult(t * (TS // 2), TS // 2)
        k = _rev_blocks(_mm(xn, _up(wkp[...]))).astype(BF16)
        kf = k[0:NVMAX * 16].astype(F32)
        for g in range(4):
            kp = _pk(k[:, g * 128:(g + 1) * 128])
            kk[g, pl.ds(p0, TS // 2), :] = kp
            kv[g, pl.ds(_mult(t * (NVMAX * 16), 16), NVMAX * 16), :] = kf[:, g * 128:(g + 1) * 128]
            if g == 0:
                hba[pl.ds(KR0 + p0, TS // 2), :] = kp
        for b in range(NVMAX):
            kb0 = _mult(KB0 + (t * NVMAX + b) * (DH * 16), 16)
            for d in range(DH):
                hba[pl.ds(kb0 + d * 16, 16), :] = jnp.broadcast_to(kf[b * 16:(b + 1) * 16, d:d + 1], (16, 128))

    def q_store(qf, t):
        q = (qf * QSCALE).astype(BF16)
        qt[:, pl.ds(_mult(t * TS, TS), TS)] = _pk(q)
        qe[:, pl.ds(_mult(t * (DH * 8), DH * 8), DH * 8), :] = jnp.broadcast_to(
            q.astype(F32)[:, None, :], (D, 8, TS)).reshape(H, DH * 8, TS)

    def v_store(v, t):
        vt[:, pl.ds(_mult(t * TS, TS), TS)] = _pk(v.astype(BF16))
        vsum[...] = vsum[...] + jnp.sum(jnp.abs(v).reshape(D // 32, 32, TS), axis=0)

    def qv_proj(xn, t):
        qv = _nt(_up(wqvt[...]), xn)
        q_store(qv[:D], t)
        v_store(qv[D:], t)

    def ln_in(b):
        for s in range(NSUB):
            r0 = _mult(b * TB + s * TS, TS)
            on[s] = _pk(_ln(xin[pl.ds(r0, TS), :].astype(F32)).astype(BF16))

    def qkv_block(b, carry):
        @pl.when(b + 1 < NB)
        def _():
            x_copy(b + 1).wait()
        for s in range(NSUB):
            k_proj(_up(on[s]), b * NSUB + s)
            qv_proj(_up(on[s]), b * NSUB + s)
        ln_in(jnp.minimum(b + 1, NB - 1))
        return carry

    def prep_piece(h, hb, k):
        g = lax.shift_right_logical(h, 3)
        lane0 = (h & 7) * DH
        rot = (lax.broadcasted_iota(jnp.int32, (8, 128), 1) + lane0) & 127
        for row in (k * 16, k * 16 + 8):
            hb[KR0 + row:KR0 + row + 8, :] = jnp.take_along_axis(
                kk[g, row:row + 8, :], rot, axis=1, mode="promise_in_bounds")
        d, i = divmod(k, 4)
        idx = jnp.full((8, 128), lane0 + d, jnp.int32)
        for c in range(4 * i, 4 * i + 4):
            for b in range(NVC[c]):
                for x in range(2):
                    src = (c * NVMAX + b) * 16 + x * 8
                    dst = KB0 + ((c * NVMAX + b) * DH + d) * 16 + x * 8
                    hb[dst:dst + 8, :] = jnp.take_along_axis(
                        kv[g, src:src + 8, :], idx, axis=1, mode="promise_in_bounds")

    def finish(h, j, a, l8):
        ot[pl.ds(_mult(h * DH, DH), DH), j * TQ:(j + 1) * TQ] = a
        for n in range(NCOL):
            lt[j * NCOL + n, pl.ds(_mult(h * 8, 8), 8), :] = l8[:, n * 128:(n + 1) * 128]
        chk[0] = chk[0] + l8
        chk[1] = jnp.minimum(chk[1], l8)

    def flush(h):
        a = ac[...] + _mm(_up(vt[pl.ds(_mult(h * 8, 8), 8), S - 128:S]), pc[...])
        finish(h, NQ - 1, a, lc[...])

    def fast_step(i, carry):
        heads = [NH * i + k for k in range(NH)]
        hbs = (hba, hbb)
        r0 = [pl.multiple_of(h * 8, 8) for h in heads]
        pblk, lsum, acc, done, snap = {}, {}, {}, {}, {}
        zz = [pl.multiple_of(zs[n] * 256, 256) for n in range(NCOL + 2)]

        def ladd(u, n, p8):
            l = lsum.get((u, n))
            if l is None:
                l = zer[0:8, 0:128]
            lsum[(u, n)] = l + p8

        def vpu_part(t, n, b, halves):
            u, c = divmod(t, NC)
            k = t // T
            sv = None
            for d0 in range(0, DH, DG):
                row = (((u % NQ) * NCOL + n) * DH + d0) * 8
                q8 = (qe[heads[k], pl.ds(row + zz[NCOL + 1], DG * 8), :] if b
                      else qe[heads[k], row:row + DG * 8, :]).reshape(DG, 1, 8, 128)
                if t == TT - 1:
                    q8 = jnp.where(snap[n] < 0.0, 0.0, q8)
                kb = hbs[k][pl.ds(KB0 + ((c * NVMAX + b) * DH + d0) * 16 + zz[n], DG * 16), :]
                kb = kb.reshape(DG, 2, 8, 128)
                if len(halves) == 1:
                    kb = kb[:, halves[0]:halves[0] + 1]
                pr = kb * q8
                if sv is not None:
                    pr = jnp.concatenate([sv[None], pr], axis=0)
                sv = jnp.sum(pr, axis=0)
            for m, x in enumerate(halves):
                p = jnp.exp2(sv[m])
                ladd(u, n, p)
                if t == TT - 2:
                    snap[n] = lsum[(u, n)]
                pblk[(t, b, n, x)] = p
                if u > 0 and not done.get((u - 1, n)):
                    lsum[(u - 1, n)] = jnp.where(p < 0.0, p, lsum[(u - 1, n)])

        def dot_blocks(blist, vsched):
            if not blist:
                return
            u = blist[0][0] // NC
            k, j = divmod(u, NQ)
            w = jnp.concatenate(
                [_up(qt[pl.ds(r0[k], 8), j * TQ:(j + 1) * TQ]), jnp.zeros((128 - DH, TQ), BF16)], axis=0)
            kc = _up(jnp.concatenate(
                [hbs[k][pl.ds(KR0 + (t % NC) * 64 + b * 8 + zz[NCOL], 8), :] for (t, b) in blist], axis=0))
            s = _mm(kc, w)
            for m, (t, b) in enumerate(blist):
                for f in vsched.pop(0):
                    f()
                p = jnp.exp2(s[m * 16:(m + 1) * 16])
                for n in range(NCOL):
                    for x in range(2):
                        p8 = p[x * 8:(x + 1) * 8, n * 128:(n + 1) * 128]
                        ladd(u, n, p8)
                        pblk[(t, b, n, x)] = p8
                    if t % NC == NC - 1 and b == 7:
                        done[(u, n)] = True

        def qk(t):
            l0 = [(t - 1, b) for b in range(NV[t - 1] + OFF, 8)] if t >= 1 else []
            l1 = [(t, b) for b in range(NV[t], NV[t] + OFF)] if t < TT else []
            nb = len(l0) + len(l1)
            vs = [[] for _ in range(nb)]
            parts = [(t, n, 0, VPOS[n], (0, 1)) for n in range(NCOL)] if t < TT else []
            for (tt, n, b, pos, halves) in parts + XS[t]:
                vs[min(pos, nb - 1)].append(functools.partial(vpu_part, tt, n, b, halves))
            if t % NC:
                dot_blocks(l0 + l1, vs)
            else:
                dot_blocks(l0, vs)
                dot_blocks(l1, vs)

        def ptile(t):
            return jnp.concatenate([
                jnp.concatenate([pblk.pop((t, b, n, x)) for n in range(NCOL)], axis=1)
                for b in reversed(range(8)) for x in (1, 0)], axis=0)

        def lrow(u):
            return jnp.concatenate([lsum[(u, n)] for n in range(NCOL)], axis=1)

        def pv(t):
            u, c = divmod(t, NC)
            k, j = divmod(u, NQ)
            a = acc.get(u)
            if a is None:
                a = zer[...]
            a = a + _mm(_up(vt[pl.ds(r0[k], 8), c * 128:(c + 1) * 128]), ptile(t))
            acc[u] = a
            if c == NC - 1:
                finish(heads[k], j, a, lrow(u))

        for t in range(TT + 1):
            qk(t)
            if t == 1:
                flush(jnp.maximum(heads[0] - 1, 0))
            if t >= 2:
                pv(t - 2)
            k, tl = divmod(t, T)
            if k < NH and tl * PPP < T:
                for m in range(PPP):
                    prep_piece(jnp.minimum(heads[k] + 1, H - 1), hbs[(k + 1) % 2], tl * PPP + m)
        pc[...] = ptile(TT - 1)
        ac[...] = acc[NH * NQ - 1]
        lc[...] = lrow(NH * NQ - 1)
        return carry

    def safe_unit(u, carry):
        h = lax.shift_right_logical(u, 2)
        g = lax.shift_right_logical(h, 3)
        j = u & (NQ - 1)
        q0 = pl.multiple_of(j * TQ, TQ)
        rows = lax.broadcasted_iota(jnp.int32, (128, TQ), 0)
        qg = _up(qt[pl.ds(pl.multiple_of(g * 64, 64), 64), pl.ds(q0, TQ)]).astype(F32)
        w = jnp.where(lax.shift_right_logical(rows, 4) == (h & 7), qg, 0.0).astype(BF16)

        def scores(c, m):
            s = _rev_blocks(_mm(_up(kk[g, pl.ds(pl.multiple_of(c * 64, 64), 64), :]), w))
            sbuf[pl.ds(pl.multiple_of(c * 128, 128), 128), :] = s
            return jnp.maximum(m, jnp.max(s, axis=0, keepdims=True))

        m = lax.fori_loop(0, NC, scores, jnp.full((1, TQ), -jnp.inf, F32))

        def weigh(c, la):
            l, a = la
            c0 = pl.multiple_of(c * 128, 128)
            p = jnp.exp2(sbuf[pl.ds(c0, 128), :] - m)
            l = l + jnp.sum(p, axis=0, keepdims=True)
            a = a + _mm(_up(vt[pl.ds(pl.multiple_of(h * 8, 8), 8), pl.ds(c0, 128)]), p.astype(BF16))
            return l, a

        l, a = lax.fori_loop(0, NC, weigh, (jnp.zeros((1, TQ), F32), jnp.zeros((DH, TQ), F32)))
        ot[pl.ds(pl.multiple_of(h * DH, DH), DH), pl.ds(q0, TQ)] = a
        l8 = jnp.broadcast_to(l * 0.125, (8, TQ))
        for n in range(NCOL):
            lt[j * NCOL + n, pl.ds(pl.multiple_of(h * 8, 8), 8), :] = l8[:, n * 128:(n + 1) * 128]
        return carry

    def wprep(r, carry):
        r16 = pl.multiple_of(r * 16, 16)
        r8 = pl.ds(pl.multiple_of(r * 8, 8), 8)

        def two(w, row, cols):
            return jnp.concatenate([w[pl.ds(r16 + row + e * 128, 16), cols].astype(F32) for e in range(2)], axis=0)

        for sc in range(NSC + 1):
            w_ = 256 if sc < NSC else 128
            cl = slice(sc * 256, sc * 256 + w_)
            cr = slice(HF + sc * 256, HF + sc * 256 + w_)
            rg, ru = [_rhs7(two(w, 0, cl), two(w, 0, cr), two(w, HD, cl), two(w, HD, cr)) for w in (wg, wu)]
            for i in range(7):
                if sc < NSC:
                    for m, (tg, tu) in enumerate(zip(_rhs7(*_quads(rg[i])), _rhs7(*_quads(ru[i])))):
                        wgu2[(sc * 7 + i) * 7 + m, r8, :] = _pk(jnp.concatenate([tg, tu], axis=1).astype(BF16))
                else:
                    t = _pk(jnp.concatenate([rg[i], ru[i]], axis=1).astype(BF16))
                    for e in range(2):
                        wgu1[i, e, r8, :] = t[e * 8:(e + 1) * 8]
        for sc in range(NSC):
            top, bot = two(wd, sc * 256, slice(None)), two(wd, HF + sc * 256, slice(None))
            for i, t in enumerate(_rhs7(top[:, :HD], top[:, HD:], bot[:, :HD], bot[:, HD:])):
                t7 = _pk(jnp.concatenate(_rhs7(*_quads(t)), axis=1).astype(BF16))
                for j in range(7):
                    wdn2[i * 7 + j, sc, r8, :] = t7[:, j * 128:(j + 1) * 128]
        top = wd[pl.ds(r16 + NSC * 256, 16), :].astype(F32)
        bot = wd[pl.ds(r16 + HF + NSC * 256, 16), :].astype(F32)
        for i, t in enumerate(_rhs7(top[:, :HD], top[:, HD:], bot[:, :HD], bot[:, HD:])):
            wdn1[i, r8, :] = _pk(t.astype(BF16))
        wop[pl.ds(pl.multiple_of(r * 32, 32), 32), :] = _pk(wo[pl.ds(pl.multiple_of(r * 64, 64), 64), :])
        return carry

    def o_stage(b):
        for s in range(NSUB):
            cols = pl.ds(_mult(b * TB + s * TS, TS), TS)
            ct = b * NSUB + s
            den = lt[ct, pl.ds(0, H, stride=8), :]
            for i in range(1, 8):
                den = den + lt[ct, pl.ds(i, H, stride=8), :]
            r = 1.0 / den
            o = jnp.concatenate([ot[h * DH:(h + 1) * DH, cols] * r[h:h + 1] for h in range(H)], axis=0)
            on[s] = _pk(o.T.astype(BF16))

    def ffn_block(b, carry, *, first):
        r0 = [pl.multiple_of(b * TB + s * TS, TS) for s in range(NSUB)]
        zj = [zs[j] for j in range(8)]
        x1 = []
        for s in range(NSUB):
            res = xin[pl.ds(r0[s], TS), :].astype(F32) if first else xs[pl.ds(r0[s], TS), :]
            x1.append(res + _mm(_up(on[s]), _up(wop[...])))
        o_stage(jnp.minimum(b + 1, NB - 1))
        for s in range(NSUB):
            xb[s][0] = _ln(x1[s])
        la1 = [_lhs1(i, lambda q: xb[q // 2][zj[7], :, (q % 2) * HD:(q % 2 + 1) * HD]).astype(BF16)
               for i in range(7)]
        la2 = [[_lhs1(j, lambda r: _lhs1(i, lambda q: xb[q // 2][
            zj[j], (r // 2) * 64:(r // 2 + 1) * 64,
            (q % 2) * HD + (r % 2) * 128:(q % 2) * HD + (r % 2 + 1) * 128])).astype(BF16)
            for j in range(7)] for i in range(7)]

        def gu(i, sc, k):
            if sc == NSC:
                return _mm(la1[i], _up(wgu1[i].reshape(HD // 2, 256)))
            return _join(_combine7({
                j: _mm(la2[i][j], _up(wgu2[(sc * 7 + i) * 7 + j, :, k * 128:(k + 1) * 128])) for j in IN_ORDER}))

        early = {(i, sc, k): gu(i, sc, k) for (sc, k) in GU_EARLY for i in GU_ORDER[:2]}

        def outer(sc, k):
            return _combine7({i: early[(i, sc, k)] if (i, sc, k) in early else gu(i, sc, k) for i in GU_ORDER})

        for sc in range(NSC):
            for q, (g, u) in enumerate(zip(outer(sc, 0), outer(sc, 1))):
                hs[q, :, sc * 256:(sc + 1) * 256] = g * u
        hodd = [t[:, :128] * t[:, 128:] for t in outer(NSC, 0)]

        def dn_lhs(i, j):
            def blk(q, r):
                rows = slice((r // 2) * 64, (r // 2 + 1) * 64)
                return jnp.concatenate(
                    [hs[q + zj[j], rows, sc * 256 + (r % 2) * 128:sc * 256 + (r % 2 + 1) * 128]
                     for sc in range(NSC)], axis=1)
            return _lhs1(j, lambda r: _lhs1(i, lambda q: blk(q, r))).astype(BF16)

        m = {}
        for i in IN_ORDER:
            inner = {j: _mm(dn_lhs(i, j), _up(wdn2[i * 7 + j].reshape(NSC * 64, 128))) for j in IN_ORDER}
            m[i] = _join(_combine7(inner)) + _mm(_lhs1(i, lambda q: hodd[q]).astype(BF16), _up(wdn1[i]))
        c = _combine7(m)
        x2 = [x1[s] + jnp.concatenate([c[2 * s], c[2 * s + 1]], axis=1) for s in range(NSUB)]
        for s in range(NSUB):
            if first:
                xs[pl.ds(r0[s], TS), :] = x2[s]
            else:
                xin[pl.ds(r0[s], TS), :] = x2[s].astype(BF16)
        if first:
            for s in range(NSUB):
                xn2 = _ln(x2[s]).astype(BF16)
                k_proj(xn2, b * NSUB + s)
                qv_proj(xn2, b * NSUB + s)
        else:
            o_copy(b).start()
        return carry

    def w_transpose(w, i):
        for j in range(4):
            wqvt[i * HD + j * 64:i * HD + (j + 1) * 64, :] = _pk(
                w[:, j * 128:(j + 1) * 128].astype(F32).T.astype(BF16))

    x_copy(0).start()
    wk_copy.start()
    zer[...] = jnp.zeros(zer.shape, zer.dtype)
    vsum[...] = jnp.zeros(vsum.shape, vsum.dtype)
    for n in range(8):
        zs[n] = 0
    x_copy(0).wait()
    wq_copy.start()
    ln_in(0)
    wk_copy.wait()
    wv_copy.start()
    x_copy(1).start()
    wkp[...] = _pk(wk[...])
    k_proj(_up(on[0]), 0)
    wq_copy.wait()
    k_proj(_up(on[1]), 1)
    w_transpose(wq, 0)
    q_store(_nt(_up(wqvt[:HD]), _up(on[0])), 0)
    wv_copy.wait()
    x_copy(1).wait()
    for b in range(2, NB):
        x_copy(b).start()
    q_store(_nt(_up(wqvt[:HD]), _up(on[1])), 1)
    w_transpose(wv, 1)
    for s in range(NSUB):
        v_store(_nt(_up(wqvt[HD:]), _up(on[s])), s)
    ln_in(1)
    for cp in w_copies:
        cp.start()
    lax.fori_loop(1, NB, qkv_block, 0)
    for cp in w_copies:
        cp.wait()
    lax.fori_loop(0, 8, wprep, 0)

    def layer(li, carry):
        chk[0] = jnp.zeros((8, TQ), F32)
        chk[1] = jnp.ones((8, TQ), F32)
        pc[...] = jnp.zeros(pc.shape, pc.dtype)
        ac[...] = jnp.zeros(ac.shape, ac.dtype)
        lc[...] = jnp.ones(lc.shape, lc.dtype)
        lax.fori_loop(0, H // NH, fast_step, 0)
        flush(H - 1)
        o_stage(0)

        vabs = jnp.concatenate([vsum[n * 8:(n + 1) * 8] for n in range(NCOL)], axis=1)
        ok = (chk[0] <= L_HI) & (chk[1] >= L_LO) & (vabs <= L_HI)

        @pl.when(jnp.max(jnp.where(ok, 0.0, 1.0)) > 0.0)
        def _():
            lax.fori_loop(0, H * NQ, safe_unit, 0)
            o_stage(0)

        @pl.when(li == 0)
        def _():
            lax.fori_loop(0, NB, functools.partial(ffn_block, first=True), 0)

        @pl.when(li == 1)
        def _():
            lax.fori_loop(0, NB, functools.partial(ffn_block, first=False), 0)
        return carry

    lax.fori_loop(0, 2, layer, 0)
    for b in range(NB):
        o_copy(b).wait()


@jax.jit
def pallas_interleave_layers__softmax_full_mha__glu_gated_bilinear__prompt_kernel(
    A_x: jax.Array,
    A_wqkv: jax.Array,
    A_wo: jax.Array,
    B_x: jax.Array,
    B_w_gate: jax.Array,
    B_w_up: jax.Array,
    B_w_down: jax.Array,
):
    del B_x
    any_spec = pl.BlockSpec(memory_space=pl.ANY)
    out = pl.pallas_call(
        _kernel,
        out_shape=jax.ShapeDtypeStruct((S, D), A_x.dtype),
        in_specs=[any_spec] * 6,
        out_specs=any_spec,
        scratch_shapes=[
            pltpu.VMEM((S, D), BF16),
            pltpu.VMEM((D, D), BF16),
            pltpu.VMEM((D, D), BF16),
            pltpu.VMEM((D, D), BF16),
            pltpu.VMEM((D, D), BF16),
            pltpu.VMEM((D, F), BF16),
            pltpu.VMEM((D, F), BF16),
            pltpu.VMEM((F, D), BF16),
            pltpu.VMEM((HD, D), F32),
            pltpu.VMEM((HD, D), F32),
            pltpu.VMEM((7, 2, 64, 256), F32),
            pltpu.VMEM((NSC * 49, 64, 256), F32),
            pltpu.VMEM((7, 64, HD), F32),
            pltpu.VMEM((49, NSC, 64, 128), F32),
            pltpu.VMEM((S, D), F32),
            pltpu.VMEM((D, D), F32),
            pltpu.VMEM((4, S // 2, 128), F32),
            pltpu.VMEM((4, NC * NVMAX * 16, 128), F32),
            pltpu.VMEM((HD, S), F32),
            pltpu.VMEM((HD, S), F32),
            pltpu.VMEM((D, S), F32),
            pltpu.VMEM((NSUB, TS // 2, D), F32),
            pltpu.VMEM((DH, TQ), F32),
            pltpu.VMEM((HB_ROWS, 128), F32),
            pltpu.VMEM((HB_ROWS, 128), F32),
            pltpu.VMEM((H, NC * DH * 8, 128), F32),
            pltpu.VMEM((NC, H * 8 + 32, 128), F32),
            pltpu.VMEM((2, 8, TQ), F32),
            pltpu.VMEM((128, TQ), F32),
            pltpu.VMEM((DH, TQ), F32),
            pltpu.VMEM((8, TQ), F32),
            pltpu.VMEM((S, TQ), F32),
            pltpu.VMEM((32, 128), F32),
            pltpu.VMEM((4, TS, NSC * 256), F32),
            pltpu.VMEM((1, TS, D), F32),
            pltpu.VMEM((1, TS, D), F32),
            pltpu.SMEM((8,), jnp.int32),
            pltpu.SemaphoreType.DMA((NB,)),
            pltpu.SemaphoreType.DMA((7,)),
            pltpu.SemaphoreType.DMA((NB,)),
        ],
        compiler_params=pltpu.CompilerParams(vmem_limit_bytes=110 * 1024 * 1024),
    )(A_x.reshape(S, D), A_wqkv, A_wo, B_w_gate, B_w_up, B_w_down)
    return out.reshape(1, S, D)
```

```python
import functools
import math

import jax
import jax.numpy as jnp
from jax import lax
import jax.experimental.pallas as pl
import jax.experimental.pallas.tpu as pltpu

S, D, H, DH, F = 2048, 512, 32, 16, 1792
EPS = 1e-5
QSCALE = (DH ** -0.5) * math.log2(math.e)
F32 = jnp.float32
BF16 = jnp.bfloat16

TB = 256
TS = 128
NSUB = TB // TS
NB = S // TB
HD = D // 2
HF = F // 2
NSC = HF // 256
GU_EARLY = ((0, 0), (0, 1), (1, 0))
GU_ORDER = (2, 4, 0, 3, 6, 1, 5)
IN_ORDER = (0, 3, 4, 6, 2, 1, 5)

TQ = 512
NQ = S // TQ
NCOL = TQ // 128
NC = S // 128
T = NQ * NC
NH = 2
TT = NH * T
OFF = 2
VPOS = (1, 2, 4, 6)
XGAPS = (3, 3, 3, 3, 4)
XPOS = (0, 3)
XSH = 2
PSTEP = 2
DG = 4
LTR = H * 8
L_LO = 2.0 ** -40
L_HI = 2.0 ** 60

NV = [1] * TT
XS = [[] for _ in range(TT + 1)]
_prev = XSH - 1
for _gap in XGAPS * (TT // sum(XGAPS)):
    _t = _prev + _gap
    if _t >= TT - 1:
        break
    NV[_t] += 1
    for _n in range(NCOL):
        for _x in range(2):
            XS[_prev + 1 + ((2 * _n + _x) * _gap) // (2 * NCOL)].append((_t, _n, NV[_t] - 1, XPOS[_x], (_x,)))
    _prev = _t
NVC = [max(NV[c::NC]) for c in range(NC)]
NVMAX = max(NVC)

XC = [c for c in range(NC) if NVC[c] > 1]
KBG = 2 * NC * NVMAX + 2


def _ln(x):
    mu = jnp.mean(x, axis=-1, keepdims=True)
    xc = x - mu
    var = jnp.mean(xc * xc, axis=-1, keepdims=True)
    return xc * lax.rsqrt(var + EPS)


def _pk(a):
    return pltpu.bitcast(a, F32)


def _up(a):
    return pltpu.bitcast(a, BF16)


def _mm(a, b):
    return lax.dot_general(a, b, (((1,), (0,)), ((), ())), preferred_element_type=F32)


def _nt(a, b):
    return lax.dot_general(a, b, (((1,), (1,)), ((), ())), preferred_element_type=F32)


def _lhs1(i, a):
    p, sign, q = ((0, 1, 3), (2, 1, 3), (0, 0, 0), (3, 0, 0), (0, 1, 1), (2, -1, 0), (1, -1, 3))[i]
    return a(p) if sign == 0 else (a(p) + a(q) if sign > 0 else a(p) - a(q))


def _rhs7(b11, b12, b21, b22):
    return [b11 + b22, b11, b12 - b22, b21 - b11, b22, b11 + b12, b21 + b22]


def _combine7(m):
    return (m[0] + m[3] - m[4] + m[6], m[2] + m[4], m[1] + m[3], m[0] - m[1] + m[2] + m[5])


def _quads(a):
    r, c = a.shape[0] // 2, a.shape[1] // 2
    return a[:r, :c], a[:r, c:], a[r:, :c], a[r:, c:]


def _join(c):
    return jnp.concatenate([jnp.concatenate(c[:2], axis=1), jnp.concatenate(c[2:], axis=1)], axis=0)


def _rev_blocks(a):
    return jnp.concatenate([a[(15 - i) * 8:(16 - i) * 8] for i in range(16)], axis=0)


def _mult(v, m):
    return v if isinstance(v, int) else pl.multiple_of(v, m)


def _kernel(x_hbm, wqkv_hbm, wo_hbm, wg_hbm, wu_hbm, wd_hbm, o_hbm,
            xin, wq, wk, wv, wo, wg, wu, wd, wkp, wop, wgu1, wgu2, wdn1, wdn2, xs, wqvt,
            kk, kv, qt, vt, ot, on, zer, kra, krb, kba, kbb, qe, lt, chk, pc, ac, lc, sbuf, vsum,
            hs, xb0, xb1, zs, sem_x, sem_w, sem_o):
    xb = (xb0, xb1)

    def x_copy(b):
        return pltpu.make_async_copy(x_hbm.at[pl.ds(b * TB, TB)], xin.at[pl.ds(b * TB, TB)], sem_x.at[b])

    def o_copy(b):
        return pltpu.make_async_copy(xin.at[pl.ds(b * TB, TB)], o_hbm.at[pl.ds(b * TB, TB)], sem_o.at[b])

    w_copies = [pltpu.make_async_copy(src, dst, sem_w.at[i]) for i, (src, dst) in enumerate(
        [(wo_hbm, wo), (wg_hbm, wg), (wu_hbm, wu), (wd_hbm, wd)])]
    wq_copy, wk_copy, wv_copy = [
        pltpu.make_async_copy(wqkv_hbm.at[:, pl.ds(i * D, D)], dst, sem_w.at[4 + i])
        for i, dst in enumerate((wq, wk, wv))]

    def k_proj(xn, t):
        p0 = _mult(t * (TS // 2), TS // 2)
        k = _rev_blocks(_mm(xn, _up(wkp[...]))).astype(BF16)
        kf = k[0:NVMAX * 16].astype(F32)
        for g in range(4):
            kp = _pk(k[:, g * 128:(g + 1) * 128])
            kk[g, pl.ds(p0, TS // 2), :] = kp
            for b in range(NVMAX):
                kv[g, b, pl.ds(_mult(t * 16, 16), 16), :] = kf[b * 16:(b + 1) * 16, g * 128:(g + 1) * 128]
            if g == 0:
                kra[pl.ds(p0, TS // 2), :] = kp
        for b in range(NVMAX):
            for d in range(DH):
                kba[d, pl.ds(2 * (b * NC + t), 2)] = jnp.broadcast_to(
                    kf[b * 16:(b + 1) * 16, d:d + 1], (16, 128)).reshape(2, 8, 128)

    def q_store(qf, t):
        q = (qf * QSCALE).astype(BF16)
        qt[:, pl.ds(_mult(t * TS, TS), TS)] = _pk(q)
        qe[:, pl.ds(t * DH, DH)] = jnp.broadcast_to(
            q.astype(F32)[:, None, :], (D, 8, TS)).reshape(H, DH, 1, 8, TS)

    def v_store(v, t):
        vt[:, pl.ds(_mult(t * TS, TS), TS)] = _pk(v.astype(BF16))
        vsum[...] = vsum[...] + jnp.sum(jnp.abs(v).reshape(D // 32, 32, TS), axis=0)

    def qv_proj(xn, t):
        qv = _nt(_up(wqvt[...]), xn)
        q_store(qv[:D], t)
        v_store(qv[D:], t)

    def ln_in(b):
        for s in range(NSUB):
            r0 = _mult(b * TB + s * TS, TS)
            on[s] = _pk(_ln(xin[pl.ds(r0, TS), :].astype(F32)).astype(BF16))

    def qkv_block(b, carry):
        @pl.when(b + 1 < NB)
        def _():
            x_copy(b + 1).wait()
        for s in range(NSUB):
            k_proj(_up(on[s]), b * NSUB + s)
            qv_proj(_up(on[s]), b * NSUB + s)
        ln_in(jnp.minimum(b + 1, NB - 1))
        return carry

    def gather(x, idx):
        return jnp.take_along_axis(x, idx, axis=1, mode="promise_in_bounds")

    def prep_piece(h, kr, kb, d):
        g = lax.shift_right_logical(h, 3)
        lane0 = (h & 7) * DH
        rows = slice(d * 64, (d + 1) * 64)
        kr[rows, :] = gather(kk[g, rows, :], (lax.broadcasted_iota(jnp.int32, (64, 128), 1) + lane0) & 127)
        src = jnp.concatenate([kv[g, 0]] + [kv[g, 1, c * 16:(c + 1) * 16, :] for c in XC], axis=0)
        col = gather(src, jnp.full(src.shape, lane0 + d, jnp.int32)).reshape(-1, 8, 128)
        kb[d, 0:2 * NC] = col[0:2 * NC]
        for m, c in enumerate(XC):
            kb[d, 2 * (NC + c):2 * (NC + c) + 2] = col[2 * (NC + m):2 * (NC + m) + 2]

    def finish(h, j, a, l8):
        ot[pl.ds(_mult(h * DH, DH), DH), j * TQ:(j + 1) * TQ] = a
        for n in range(NCOL):
            lt[pl.ds(_mult((j * NCOL + n) * LTR + h * 8, 8), 8), :] = l8[:, n * 128:(n + 1) * 128]
        chk[0] = chk[0] + l8
        chk[1] = jnp.minimum(chk[1], l8)

    def flush(h):
        a = ac[...] + _mm(_up(vt[pl.ds(_mult(h * 8, 8), 8), S - 128:S]), pc[...])
        finish(h, NQ - 1, a, lc[...])

    def fast_step(i, carry):
        heads = [NH * i + k for k in range(NH)]
        krs, kbs = (kra, krb), (kba, kbb)
        r0 = [pl.multiple_of(h * 8, 8) for h in heads]
        pblk, lsum, acc, done, snap = {}, {}, {}, {}, {}
        zz = [zs[n] * 32 for n in range(NCOL + 1)]
        heads2 = [h + zs[NCOL + 1] for h in heads]

        def ladd(u, n, p):
            l = lsum.get((u, n))
            if l is None:
                l = zer[0:8, 0:128]
            lsum[(u, n)] = jnp.sum(jnp.concatenate([l[None], p], axis=0), axis=0)

        def vpu_part(t, n, b, halves):
            u, c = divmod(t, NC)
            k = t // T
            grp = pl.ds(2 * (b * NC + c) + halves[0] + zz[n], len(halves))
            hq = heads2[k] if b else heads[k]
            sv = None
            for d0 in range(0, DH, DG):
                row = ((u % NQ) * NCOL + n) * DH + d0
                q8 = qe[hq, row:row + DG]
                if t == TT - 1:
                    q8 = jnp.where(snap[n] < 0.0, 0.0, q8)
                pr = kbs[k][d0:d0 + DG, grp] * q8
                if sv is not None:
                    pr = jnp.concatenate([sv, pr], axis=0)
                sv = jnp.sum(pr, axis=0, keepdims=d0 + DG < DH)
            p = jnp.exp2(sv)
            ladd(u, n, p)
            if t == TT - 2:
                snap[n] = lsum[(u, n)]
            for m, x in enumerate(halves):
                pm = p[m:m + 1] if len(halves) > 1 else p
                pblk[(t, b, x, n)] = pm
                if u > 0 and not done.get(u - 1):
                    lsum[(u - 1, n)] = jnp.where(pm[0] < 0.0, pm[0], lsum[(u - 1, n)])

        def dot_blocks(blist, vsched):
            if not blist:
                return
            u = blist[0][0] // NC
            k, j = divmod(u, NQ)
            w = jnp.concatenate(
                [_up(qt[pl.ds(r0[k], 8), j * TQ:(j + 1) * TQ]), jnp.zeros((128 - DH, TQ), BF16)], axis=0)
            runs = {}
            for t, b in blist:
                runs.setdefault(t, []).append(b)
            kc = _up(jnp.concatenate(
                [krs[k][pl.ds(pl.multiple_of((t % NC) * 64 + bs[0] * 8 + zz[NCOL], 8), len(bs) * 8), :]
                 for t, bs in runs.items()], axis=0))
            p = jnp.exp2(_mm(kc, w)).reshape(2 * len(blist), 8, TQ)
            for m, (t, b) in enumerate(blist):
                for x in range(2):
                    pblk[(t, b, x)] = p[2 * m + x:2 * m + x + 1]
            first = [0] * NCOL

            def catch_up(n, m):
                if m > first[n]:
                    ladd(u, n, p[2 * first[n]:2 * m, :, n * 128:(n + 1) * 128])
                    first[n] = m

            for m in range(len(blist)):
                for part in vsched.pop(0):
                    catch_up(part[1], m)
                    vpu_part(*part)
            for n in range(NCOL):
                catch_up(n, len(blist))
            if blist[-1] == (u * NC + NC - 1, 7):
                done[u] = True

        def qk(t):
            l0 = [(t - 1, b) for b in range(NV[t - 1] + OFF, 8)] if t >= 1 else []
            l1 = [(t, b) for b in range(NV[t], NV[t] + OFF)] if t < TT else []
            nb = len(l0) + len(l1)
            vs = [[] for _ in range(nb)]
            parts = [(t, n, 0, VPOS[n], (0, 1)) for n in range(NCOL)] if t < TT else []
            for (tt, n, b, pos, halves) in parts + XS[t]:
                vs[min(pos, nb - 1)].append((tt, n, b, halves))
            if t % NC:
                dot_blocks(l0 + l1, vs)
            else:
                dot_blocks(l0, vs)
                dot_blocks(l1, vs)

        def ptile(t):
            return jnp.concatenate([
                pblk.pop((t, b, x)) if b >= NV[t] else
                jnp.concatenate([pblk.pop((t, b, x, n)) for n in range(NCOL)], axis=2)
                for b in reversed(range(8)) for x in (1, 0)], axis=0).reshape(128, TQ)

        def lrow(u):
            return jnp.concatenate([lsum[(u, n)] for n in range(NCOL)], axis=1)

        def pv(t):
            u, c = divmod(t, NC)
            k, j = divmod(u, NQ)
            a = acc.get(u)
            if a is None:
                a = zer[...]
            a = a + _mm(_up(vt[pl.ds(r0[k], 8), c * 128:(c + 1) * 128]), ptile(t))
            acc[u] = a
            if c == NC - 1:
                finish(heads[k], j, a, lrow(u))

        for t in range(TT + 1):
            qk(t)
            if t == 1:
                flush(jnp.maximum(heads[0] - 1, 0))
            if t >= 2:
                pv(t - 2)
            k, tl = divmod(t, T)
            if k < NH and tl % PSTEP == 0 and tl // PSTEP < DH:
                prep_piece(jnp.minimum(heads[k] + 1, H - 1), krs[1 - k], kbs[1 - k], tl // PSTEP)
        pc[...] = ptile(TT - 1)
        ac[...] = acc[NH * NQ - 1]
        lc[...] = lrow(NH * NQ - 1)
        return carry

    def safe_unit(u, carry):
        h = lax.shift_right_logical(u, 2)
        g = lax.shift_right_logical(h, 3)
        j = u & (NQ - 1)
        q0 = pl.multiple_of(j * TQ, TQ)
        rows = lax.broadcasted_iota(jnp.int32, (128, TQ), 0)
        qg = _up(qt[pl.ds(pl.multiple_of(g * 64, 64), 64), pl.ds(q0, TQ)]).astype(F32)
        w = jnp.where(lax.shift_right_logical(rows, 4) == (h & 7), qg, 0.0).astype(BF16)

        def scores(c, m):
            s = _rev_blocks(_mm(_up(kk[g, pl.ds(pl.multiple_of(c * 64, 64), 64), :]), w))
            sbuf[pl.ds(pl.multiple_of(c * 128, 128), 128), :] = s
            return jnp.maximum(m, jnp.max(s, axis=0, keepdims=True))

        m = lax.fori_loop(0, NC, scores, jnp.full((1, TQ), -jnp.inf, F32))

        def weigh(c, la):
            l, a = la
            c0 = pl.multiple_of(c * 128, 128)
            p = jnp.exp2(sbuf[pl.ds(c0, 128), :] - m)
            l = l + jnp.sum(p, axis=0, keepdims=True)
            a = a + _mm(_up(vt[pl.ds(pl.multiple_of(h * 8, 8), 8), pl.ds(c0, 128)]), p.astype(BF16))
            return l, a

        l, a = lax.fori_loop(0, NC, weigh, (jnp.zeros((1, TQ), F32), jnp.zeros((DH, TQ), F32)))
        ot[pl.ds(pl.multiple_of(h * DH, DH), DH), pl.ds(q0, TQ)] = a
        l8 = jnp.broadcast_to(l * 0.125, (8, TQ))
        for n in range(NCOL):
            lt[pl.ds(pl.multiple_of((j * NCOL + n) * LTR + h * 8, 8), 8), :] = l8[:, n * 128:(n + 1) * 128]
        return carry

    def wprep(r, carry):
        r16 = pl.multiple_of(r * 16, 16)
        r8 = pl.ds(pl.multiple_of(r * 8, 8), 8)

        def two(w, row, cols):
            return jnp.concatenate([w[pl.ds(r16 + row + e * 128, 16), cols].astype(F32) for e in range(2)], axis=0)

        for sc in range(NSC + 1):
            w_ = 256 if sc < NSC else 128
            cl = slice(sc * 256, sc * 256 + w_)
            cr = slice(HF + sc * 256, HF + sc * 256 + w_)
            rg, ru = [_rhs7(two(w, 0, cl), two(w, 0, cr), two(w, HD, cl), two(w, HD, cr)) for w in (wg, wu)]
            for i in range(7):
                if sc < NSC:
                    for m, (tg, tu) in enumerate(zip(_rhs7(*_quads(rg[i])), _rhs7(*_quads(ru[i])))):
                        wgu2[(sc * 7 + i) * 7 + m, r8, :] = _pk(jnp.concatenate([tg, tu], axis=1).astype(BF16))
                else:
                    t = _pk(jnp.concatenate([rg[i], ru[i]], axis=1).astype(BF16))
                    for e in range(2):
                        wgu1[i, e, r8, :] = t[e * 8:(e + 1) * 8]
        for sc in range(NSC):
            top, bot = two(wd, sc * 256, slice(None)), two(wd, HF + sc * 256, slice(None))
            for i, t in enumerate(_rhs7(top[:, :HD], top[:, HD:], bot[:, :HD], bot[:, HD:])):
                t7 = _pk(jnp.concatenate(_rhs7(*_quads(t)), axis=1).astype(BF16))
                for j in range(7):
                    wdn2[i * 7 + j, sc, r8, :] = t7[:, j * 128:(j + 1) * 128]
        top = wd[pl.ds(r16 + NSC * 256, 16), :].astype(F32)
        bot = wd[pl.ds(r16 + HF + NSC * 256, 16), :].astype(F32)
        for i, t in enumerate(_rhs7(top[:, :HD], top[:, HD:], bot[:, :HD], bot[:, HD:])):
            wdn1[i, r8, :] = _pk(t.astype(BF16))
        wop[pl.ds(pl.multiple_of(r * 32, 32), 32), :] = _pk(wo[pl.ds(pl.multiple_of(r * 64, 64), 64), :])
        return carry

    def o_stage(b):
        for s in range(NSUB):
            cols = pl.ds(_mult(b * TB + s * TS, TS), TS)
            l0 = (b * NSUB + s) * LTR
            den = lt[pl.ds(l0, H, stride=8), :]
            for i in range(1, 8):
                den = den + lt[pl.ds(l0 + i, H, stride=8), :]
            r = 1.0 / den
            o = jnp.concatenate([ot[h * DH:(h + 1) * DH, cols] * r[h:h + 1] for h in range(H)], axis=0)
            on[s] = _pk(o.T.astype(BF16))

    def ffn_block(b, carry, *, first):
        r0 = [pl.multiple_of(b * TB + s * TS, TS) for s in range(NSUB)]
        zj = [zs[j] for j in range(8)]
        x1 = []
        for s in range(NSUB):
            res = xin[pl.ds(r0[s], TS), :].astype(F32) if first else xs[pl.ds(r0[s], TS), :]
            x1.append(res + _mm(_up(on[s]), _up(wop[...])))
        o_stage(jnp.minimum(b + 1, NB - 1))
        for s in range(NSUB):
            xb[s][0] = _ln(x1[s])
        la1 = [_lhs1(i, lambda q: xb[q // 2][zj[7], :, (q % 2) * HD:(q % 2 + 1) * HD]).astype(BF16)
               for i in range(7)]
        la2 = [[_lhs1(j, lambda r: _lhs1(i, lambda q: xb[q // 2][
            zj[j], (r // 2) * 64:(r // 2 + 1) * 64,
            (q % 2) * HD + (r % 2) * 128:(q % 2) * HD + (r % 2 + 1) * 128])).astype(BF16)
            for j in range(7)] for i in range(7)]

        def gu(i, sc, k):
            if sc == NSC:
                return _mm(la1[i], _up(wgu1[i].reshape(HD // 2, 256)))
            return _join(_combine7({
                j: _mm(la2[i][j], _up(wgu2[(sc * 7 + i) * 7 + j, :, k * 128:(k + 1) * 128])) for j in IN_ORDER}))

        early = {(i, sc, k): gu(i, sc, k) for (sc, k) in GU_EARLY for i in GU_ORDER[:2]}

        def outer(sc, k):
            return _combine7({i: early[(i, sc, k)] if (i, sc, k) in early else gu(i, sc, k) for i in GU_ORDER})

        for sc in range(NSC):
            for q, (g, u) in enumerate(zip(outer(sc, 0), outer(sc, 1))):
                hs[q, :, sc * 256:(sc + 1) * 256] = g * u
        hodd = [t[:, :128] * t[:, 128:] for t in outer(NSC, 0)]

        def dn_lhs(i, j):
            def blk(q, r):
                rows = slice((r // 2) * 64, (r // 2 + 1) * 64)
                return jnp.concatenate(
                    [hs[q + zj[j], rows, sc * 256 + (r % 2) * 128:sc * 256 + (r % 2 + 1) * 128]
                     for sc in range(NSC)], axis=1)
            return _lhs1(j, lambda r: _lhs1(i, lambda q: blk(q, r))).astype(BF16)

        m = {}
        for i in IN_ORDER:
            inner = {j: _mm(dn_lhs(i, j), _up(wdn2[i * 7 + j].reshape(NSC * 64, 128))) for j in IN_ORDER}
            m[i] = _join(_combine7(inner)) + _mm(_lhs1(i, lambda q: hodd[q]).astype(BF16), _up(wdn1[i]))
        c = _combine7(m)
        x2 = [x1[s] + jnp.concatenate([c[2 * s], c[2 * s + 1]], axis=1) for s in range(NSUB)]
        for s in range(NSUB):
            if first:
                xs[pl.ds(r0[s], TS), :] = x2[s]
            else:
                xin[pl.ds(r0[s], TS), :] = x2[s].astype(BF16)
        if first:
            for s in range(NSUB):
                xn2 = _ln(x2[s]).astype(BF16)
                k_proj(xn2, b * NSUB + s)
                qv_proj(xn2, b * NSUB + s)
        else:
            o_copy(b).start()
        return carry

    def w_transpose(w, i):
        for j in range(4):
            wqvt[i * HD + j * 64:i * HD + (j + 1) * 64, :] = _pk(
                w[:, j * 128:(j + 1) * 128].astype(F32).T.astype(BF16))

    x_copy(0).start()
    wk_copy.start()
    zer[...] = jnp.zeros(zer.shape, zer.dtype)
    vsum[...] = jnp.zeros(vsum.shape, vsum.dtype)
    for n in range(8):
        zs[n] = 0
    x_copy(0).wait()
    wq_copy.start()
    ln_in(0)
    wk_copy.wait()
    wv_copy.start()
    x_copy(1).start()
    wkp[...] = _pk(wk[...])
    k_proj(_up(on[0]), 0)
    wq_copy.wait()
    k_proj(_up(on[1]), 1)
    w_transpose(wq, 0)
    q_store(_nt(_up(wqvt[:HD]), _up(on[0])), 0)
    wv_copy.wait()
    x_copy(1).wait()
    for b in range(2, NB):
        x_copy(b).start()
    q_store(_nt(_up(wqvt[:HD]), _up(on[1])), 1)
    w_transpose(wv, 1)
    for s in range(NSUB):
        v_store(_nt(_up(wqvt[HD:]), _up(on[s])), s)
    ln_in(1)
    for cp in w_copies:
        cp.start()
    lax.fori_loop(1, NB, qkv_block, 0)
    for cp in w_copies:
        cp.wait()
    lax.fori_loop(0, 8, wprep, 0)

    def layer(li, carry):
        chk[0] = jnp.zeros((8, TQ), F32)
        chk[1] = jnp.ones((8, TQ), F32)
        pc[...] = jnp.zeros(pc.shape, pc.dtype)
        ac[...] = jnp.zeros(ac.shape, ac.dtype)
        lc[...] = jnp.ones(lc.shape, lc.dtype)
        lax.fori_loop(0, H // NH, fast_step, 0)
        flush(H - 1)
        o_stage(0)

        vabs = jnp.concatenate([vsum[n * 8:(n + 1) * 8] for n in range(NCOL)], axis=1)
        ok = (chk[0] <= L_HI) & (chk[1] >= L_LO) & (vabs <= L_HI)

        @pl.when(jnp.max(jnp.where(ok, 0.0, 1.0)) > 0.0)
        def _():
            lax.fori_loop(0, H * NQ, safe_unit, 0)
            o_stage(0)

        @pl.when(li == 0)
        def _():
            lax.fori_loop(0, NB, functools.partial(ffn_block, first=True), 0)

        @pl.when(li == 1)
        def _():
            lax.fori_loop(0, NB, functools.partial(ffn_block, first=False), 0)
        return carry

    lax.fori_loop(0, 2, layer, 0)
    for b in range(NB):
        o_copy(b).wait()


@jax.jit
def pallas_interleave_layers__softmax_full_mha__glu_gated_bilinear__prompt_kernel(
    A_x: jax.Array,
    A_wqkv: jax.Array,
    A_wo: jax.Array,
    B_x: jax.Array,
    B_w_gate: jax.Array,
    B_w_up: jax.Array,
    B_w_down: jax.Array,
):
    del B_x
    any_spec = pl.BlockSpec(memory_space=pl.ANY)
    out = pl.pallas_call(
        _kernel,
        out_shape=jax.ShapeDtypeStruct((S, D), A_x.dtype),
        in_specs=[any_spec] * 6,
        out_specs=any_spec,
        scratch_shapes=[
            pltpu.VMEM((S, D), BF16),
            pltpu.VMEM((D, D), BF16),
            pltpu.VMEM((D, D), BF16),
            pltpu.VMEM((D, D), BF16),
            pltpu.VMEM((D, D), BF16),
            pltpu.VMEM((D, F), BF16),
            pltpu.VMEM((D, F), BF16),
            pltpu.VMEM((F, D), BF16),
            pltpu.VMEM((HD, D), F32),
            pltpu.VMEM((HD, D), F32),
            pltpu.VMEM((7, 2, 64, 256), F32),
            pltpu.VMEM((NSC * 49, 64, 256), F32),
            pltpu.VMEM((7, 64, HD), F32),
            pltpu.VMEM((49, NSC, 64, 128), F32),
            pltpu.VMEM((S, D), F32),
            pltpu.VMEM((D, D), F32),
            pltpu.VMEM((4, S // 2, 128), F32),
            pltpu.VMEM((4, NVMAX, NC * 16, 128), F32),
            pltpu.VMEM((HD, S), F32),
            pltpu.VMEM((HD, S), F32),
            pltpu.VMEM((D, S), F32),
            pltpu.VMEM((NSUB, TS // 2, D), F32),
            pltpu.VMEM((DH, TQ), F32),
            pltpu.VMEM((S // 2, 128), F32),
            pltpu.VMEM((S // 2, 128), F32),
            pltpu.VMEM((DH, KBG, 8, 128), F32),
            pltpu.VMEM((DH, KBG, 8, 128), F32),
            pltpu.VMEM((H, NC * DH, 1, 8, 128), F32),
            pltpu.VMEM((NC * LTR + 32, 128), F32),
            pltpu.VMEM((2, 8, TQ), F32),
            pltpu.VMEM((128, TQ), F32),
            pltpu.VMEM((DH, TQ), F32),
            pltpu.VMEM((8, TQ), F32),
            pltpu.VMEM((S, TQ), F32),
            pltpu.VMEM((32, 128), F32),
            pltpu.VMEM((4, TS, NSC * 256), F32),
            pltpu.VMEM((1, TS, D), F32),
            pltpu.VMEM((1, TS, D), F32),
            pltpu.SMEM((8,), jnp.int32),
            pltpu.SemaphoreType.DMA((NB,)),
            pltpu.SemaphoreType.DMA((7,)),
            pltpu.SemaphoreType.DMA((NB,)),
        ],
        compiler_params=pltpu.CompilerParams(vmem_limit_bytes=110 * 1024 * 1024),
    )(A_x.reshape(S, D), A_wqkv, A_wo, B_w_gate, B_w_up, B_w_down)
    return out.reshape(1, S, D)
```

```python
import math

import jax
import jax.numpy as jnp
from jax import lax
import jax.experimental.pallas as pl
import jax.experimental.pallas.tpu as pltpu

S, D, H, DH, F = 2048, 512, 32, 16, 1792
EPS = 1e-5
QSCALE = (DH ** -0.5) * math.log2(math.e)
F32 = jnp.float32
BF16 = jnp.bfloat16

TB = 256
TS = 128
NSUB = TB // TS
NB = S // TB
HD = D // 2
HF = F // 2
NSC = HF // 256
GU_EARLY = ((0, 0), (0, 1), (3, 0))
GU_ORDER = (2, 4, 0, 3, 6, 1, 5)
IN_ORDER = (0, 3, 4, 6, 2, 1, 5)

TQ = 512
NQ = S // TQ
NCOL = TQ // 128
NC = S // 128
T = NQ * NC
NH = 2
TT = NH * T
OFF = 2
VPOS = (1, 2, 4, 6)
XGAPS = (3, 3, 3, 3, 4)
XPOS = (0, 3)
XSH = 2
PSTEP = 2
DG = 4
LTR = H * 8
L_LO = 2.0 ** -40
L_HI = 2.0 ** 60

NV = [1] * TT
XS = [[] for _ in range(TT + 1)]
_prev = XSH - 1
for _gap in XGAPS * (TT // sum(XGAPS)):
    _t = _prev + _gap
    if _t >= TT - 1:
        break
    NV[_t] += 1
    for _n in range(NCOL):
        for _x in range(2):
            XS[_prev + 1 + ((2 * _n + _x) * _gap) // (2 * NCOL)].append((_t, _n, NV[_t] - 1, XPOS[_x], (_x,)))
    _prev = _t
NVC = [max(NV[c::NC]) for c in range(NC)]
NVMAX = max(NVC)

XC = [c for c in range(NC) if NVC[c] > 1]
KBG = 2 * NC * NVMAX + 2


def _ln(x):
    mu = jnp.mean(x, axis=-1, keepdims=True)
    xc = x - mu
    var = jnp.mean(xc * xc, axis=-1, keepdims=True)
    return xc * lax.rsqrt(var + EPS)


def _pk(a):
    return pltpu.bitcast(a, F32)


def _up(a):
    return pltpu.bitcast(a, BF16)


def _mm(a, b):
    return lax.dot_general(a, b, (((1,), (0,)), ((), ())), preferred_element_type=F32)


def _nt(a, b):
    return lax.dot_general(a, b, (((1,), (1,)), ((), ())), preferred_element_type=F32)


def _lhs1(i, a):
    p, sign, q = ((0, 1, 3), (2, 1, 3), (0, 0, 0), (3, 0, 0), (0, 1, 1), (2, -1, 0), (1, -1, 3))[i]
    return a(p) if sign == 0 else (a(p) + a(q) if sign > 0 else a(p) - a(q))


def _rhs7(b11, b12, b21, b22):
    return [b11 + b22, b11, b12 - b22, b21 - b11, b22, b11 + b12, b21 + b22]


def _combine7(m):
    return (m[0] + m[3] - m[4] + m[6], m[2] + m[4], m[1] + m[3], m[0] - m[1] + m[2] + m[5])


def _quads(a):
    r, c = a.shape[0] // 2, a.shape[1] // 2
    return a[:r, :c], a[:r, c:], a[r:, :c], a[r:, c:]


def _join(c):
    return jnp.concatenate([jnp.concatenate(c[:2], axis=1), jnp.concatenate(c[2:], axis=1)], axis=0)


def _rev_blocks(a):
    return jnp.concatenate([a[(15 - i) * 8:(16 - i) * 8] for i in range(16)], axis=0)


def _mult(v, m):
    return v if isinstance(v, int) else pl.multiple_of(v, m)


def _kernel(x_hbm, wqkv_hbm, wo_hbm, wg_hbm, wu_hbm, wd_hbm, o_hbm,
            xin, wq, wk, wv, wo, wg, wu, wd, wkp, wop, wgu1, wgu2, wdn1, wdn2, xs, wqvt,
            kk, kv, qt, vt, ot, on, zer, kra, krb, kba, kbb, qe, lt, chk, pc, ac, lc, sbuf, vsum,
            hs0, hs1, xb0, xb1, xb2, xb3, zs, sem_x, sem_w, sem_o):
    def x_copy(b):
        return pltpu.make_async_copy(x_hbm.at[pl.ds(b * TB, TB)], xin.at[pl.ds(b * TB, TB)], sem_x.at[b])

    def o_copy(b):
        return pltpu.make_async_copy(xin.at[pl.ds(b * TB, TB)], o_hbm.at[pl.ds(b * TB, TB)], sem_o.at[b])

    w_copies = [pltpu.make_async_copy(src, dst, sem_w.at[i]) for i, (src, dst) in enumerate(
        [(wo_hbm, wo), (wg_hbm, wg), (wu_hbm, wu), (wd_hbm, wd)])]
    wq_copy, wk_copy, wv_copy = [
        pltpu.make_async_copy(wqkv_hbm.at[:, pl.ds(i * D, D)], dst, sem_w.at[4 + i])
        for i, dst in enumerate((wq, wk, wv))]

    def k_proj(xn, t):
        p0 = _mult(t * (TS // 2), TS // 2)
        k = _rev_blocks(_mm(xn, _up(wkp[...]))).astype(BF16)
        kf = k[0:NVMAX * 16].astype(F32)
        for g in range(4):
            kp = _pk(k[:, g * 128:(g + 1) * 128])
            kk[g, pl.ds(p0, TS // 2), :] = kp
            for b in range(NVMAX):
                kv[g, b, pl.ds(_mult(t * 16, 16), 16), :] = kf[b * 16:(b + 1) * 16, g * 128:(g + 1) * 128]
            if g == 0:
                kra[pl.ds(p0, TS // 2), :] = kp
        for b in range(NVMAX):
            for d in range(DH):
                kba[d, pl.ds(2 * (b * NC + t), 2)] = jnp.broadcast_to(
                    kf[b * 16:(b + 1) * 16, d:d + 1], (16, 128)).reshape(2, 8, 128)

    def q_store(qf, t):
        q = (qf * QSCALE).astype(BF16)
        qt[:, pl.ds(_mult(t * TS, TS), TS)] = _pk(q)
        qe[:, pl.ds(t * DH, DH)] = jnp.broadcast_to(
            q.astype(F32)[:, None, :], (D, 8, TS)).reshape(H, DH, 1, 8, TS)

    def v_store(v, t):
        vt[:, pl.ds(_mult(t * TS, TS), TS)] = _pk(v.astype(BF16))
        vsum[...] = vsum[...] + jnp.sum(jnp.abs(v).reshape(D // 32, 32, TS), axis=0)

    def qv_proj(xn, t):
        qv = _nt(_up(wqvt[...]), xn)
        q_store(qv[:D], t)
        v_store(qv[D:], t)

    def ln_in(b):
        for s in range(NSUB):
            r0 = _mult(b * TB + s * TS, TS)
            on[s] = _pk(_ln(xin[pl.ds(r0, TS), :].astype(F32)).astype(BF16))

    def qkv_block(b, carry):
        @pl.when(b + 1 < NB)
        def _():
            x_copy(b + 1).wait()
        for s in range(NSUB):
            k_proj(_up(on[s]), b * NSUB + s)
            qv_proj(_up(on[s]), b * NSUB + s)
        ln_in(jnp.minimum(b + 1, NB - 1))
        return carry

    def gather(x, idx):
        return jnp.take_along_axis(x, idx, axis=1, mode="promise_in_bounds")

    def prep_piece(h, kr, kb, d):
        g = lax.shift_right_logical(h, 3)
        lane0 = (h & 7) * DH
        rows = slice(d * 64, (d + 1) * 64)
        kr[rows, :] = gather(kk[g, rows, :], (lax.broadcasted_iota(jnp.int32, (64, 128), 1) + lane0) & 127)
        src = jnp.concatenate([kv[g, 0]] + [kv[g, 1, c * 16:(c + 1) * 16, :] for c in XC], axis=0)
        col = gather(src, jnp.full(src.shape, lane0 + d, jnp.int32)).reshape(-1, 8, 128)
        kb[d, 0:2 * NC] = col[0:2 * NC]
        for m, c in enumerate(XC):
            kb[d, 2 * (NC + c):2 * (NC + c) + 2] = col[2 * (NC + m):2 * (NC + m) + 2]

    def finish(h, j, a, l8):
        ot[pl.ds(_mult(h * DH, DH), DH), j * TQ:(j + 1) * TQ] = a
        for n in range(NCOL):
            lt[pl.ds(_mult((j * NCOL + n) * LTR + h * 8, 8), 8), :] = l8[:, n * 128:(n + 1) * 128]
        chk[0] = chk[0] + l8
        chk[1] = jnp.minimum(chk[1], l8)

    def flush(h):
        a = ac[...] + _mm(_up(vt[pl.ds(_mult(h * 8, 8), 8), S - 128:S]), pc[...])
        finish(h, NQ - 1, a, lc[...])

    def fast_step(i, carry):
        heads = [NH * i + k for k in range(NH)]
        krs, kbs = (kra, krb), (kba, kbb)
        r0 = [pl.multiple_of(h * 8, 8) for h in heads]
        pblk, lsum, acc, done, snap = {}, {}, {}, {}, {}
        zz = [zs[n] * 32 for n in range(NCOL + 1)]
        heads2 = [h + zs[NCOL + 1] for h in heads]

        def ladd(u, n, p):
            l = lsum.get((u, n))
            if l is None:
                l = zer[0:8, 0:128]
            lsum[(u, n)] = jnp.sum(jnp.concatenate([l[None], p], axis=0), axis=0)

        def vpu_part(t, n, b, halves):
            u, c = divmod(t, NC)
            k = t // T
            grp = pl.ds(2 * (b * NC + c) + halves[0] + zz[n], len(halves))
            hq = heads2[k] if b else heads[k]
            sv = None
            for d0 in range(0, DH, DG):
                row = ((u % NQ) * NCOL + n) * DH + d0
                q8 = qe[hq, row:row + DG]
                if t == TT - 1:
                    q8 = jnp.where(snap[n] < 0.0, 0.0, q8)
                pr = kbs[k][d0:d0 + DG, grp] * q8
                if sv is not None:
                    pr = jnp.concatenate([sv, pr], axis=0)
                sv = jnp.sum(pr, axis=0, keepdims=d0 + DG < DH)
            p = jnp.exp2(sv)
            ladd(u, n, p)
            if t == TT - 2:
                snap[n] = lsum[(u, n)]
            for m, x in enumerate(halves):
                pm = p[m:m + 1] if len(halves) > 1 else p
                pblk[(t, b, x, n)] = pm
                if u > 0 and not done.get(u - 1):
                    lsum[(u - 1, n)] = jnp.where(pm[0] < 0.0, pm[0], lsum[(u - 1, n)])

        def dot_blocks(blist, vsched):
            if not blist:
                return
            u = blist[0][0] // NC
            k, j = divmod(u, NQ)
            w = jnp.concatenate(
                [_up(qt[pl.ds(r0[k], 8), j * TQ:(j + 1) * TQ]), jnp.zeros((128 - DH, TQ), BF16)], axis=0)
            runs = {}
            for t, b in blist:
                runs.setdefault(t, []).append(b)
            kc = _up(jnp.concatenate(
                [krs[k][pl.ds(pl.multiple_of((t % NC) * 64 + bs[0] * 8 + zz[NCOL], 8), len(bs) * 8), :]
                 for t, bs in runs.items()], axis=0))
            p = jnp.exp2(_mm(kc, w)).reshape(2 * len(blist), 8, TQ)
            for m, (t, b) in enumerate(blist):
                for x in range(2):
                    pblk[(t, b, x)] = p[2 * m + x:2 * m + x + 1]
            first = [0] * NCOL

            def catch_up(n, m):
                if m > first[n]:
                    ladd(u, n, p[2 * first[n]:2 * m, :, n * 128:(n + 1) * 128])
                    first[n] = m

            for m in range(len(blist)):
                for part in vsched.pop(0):
                    catch_up(part[1], m)
                    vpu_part(*part)
            for n in range(NCOL):
                catch_up(n, len(blist))
            if blist[-1] == (u * NC + NC - 1, 7):
                done[u] = True

        def qk(t):
            l0 = [(t - 1, b) for b in range(NV[t - 1] + OFF, 8)] if t >= 1 else []
            l1 = [(t, b) for b in range(NV[t], NV[t] + OFF)] if t < TT else []
            nb = len(l0) + len(l1)
            vs = [[] for _ in range(nb)]
            parts = [(t, n, 0, VPOS[n], (0, 1)) for n in range(NCOL)] if t < TT else []
            for (tt, n, b, pos, halves) in parts + XS[t]:
                vs[min(pos, nb - 1)].append((tt, n, b, halves))
            if t % NC:
                dot_blocks(l0 + l1, vs)
            else:
                dot_blocks(l0, vs)
                dot_blocks(l1, vs)

        def ptile(t):
            return jnp.concatenate([
                pblk.pop((t, b, x)) if b >= NV[t] else
                jnp.concatenate([pblk.pop((t, b, x, n)) for n in range(NCOL)], axis=2)
                for b in reversed(range(8)) for x in (1, 0)], axis=0).reshape(128, TQ)

        def lrow(u):
            return jnp.concatenate([lsum[(u, n)] for n in range(NCOL)], axis=1)

        def pv(t):
            u, c = divmod(t, NC)
            k, j = divmod(u, NQ)
            a = acc.get(u)
            if a is None:
                a = zer[...]
            a = a + _mm(_up(vt[pl.ds(r0[k], 8), c * 128:(c + 1) * 128]), ptile(t))
            acc[u] = a
            if c == NC - 1:
                finish(heads[k], j, a, lrow(u))

        for t in range(TT + 1):
            qk(t)
            if t == 1:
                flush(jnp.maximum(heads[0] - 1, 0))
            if t >= 2:
                pv(t - 2)
            k, tl = divmod(t, T)
            if k < NH and tl % PSTEP == 0 and tl // PSTEP < DH:
                prep_piece(jnp.minimum(heads[k] + 1, H - 1), krs[1 - k], kbs[1 - k], tl // PSTEP)
        pc[...] = ptile(TT - 1)
        ac[...] = acc[NH * NQ - 1]
        lc[...] = lrow(NH * NQ - 1)
        return carry

    def safe_unit(u, carry):
        h = lax.shift_right_logical(u, 2)
        g = lax.shift_right_logical(h, 3)
        j = u & (NQ - 1)
        q0 = pl.multiple_of(j * TQ, TQ)
        rows = lax.broadcasted_iota(jnp.int32, (128, TQ), 0)
        qg = _up(qt[pl.ds(pl.multiple_of(g * 64, 64), 64), pl.ds(q0, TQ)]).astype(F32)
        w = jnp.where(lax.shift_right_logical(rows, 4) == (h & 7), qg, 0.0).astype(BF16)

        def scores(c, m):
            s = _rev_blocks(_mm(_up(kk[g, pl.ds(pl.multiple_of(c * 64, 64), 64), :]), w))
            sbuf[pl.ds(pl.multiple_of(c * 128, 128), 128), :] = s
            return jnp.maximum(m, jnp.max(s, axis=0, keepdims=True))

        m = lax.fori_loop(0, NC, scores, jnp.full((1, TQ), -jnp.inf, F32))

        def weigh(c, la):
            l, a = la
            c0 = pl.multiple_of(c * 128, 128)
            p = jnp.exp2(sbuf[pl.ds(c0, 128), :] - m)
            l = l + jnp.sum(p, axis=0, keepdims=True)
            a = a + _mm(_up(vt[pl.ds(pl.multiple_of(h * 8, 8), 8), pl.ds(c0, 128)]), p.astype(BF16))
            return l, a

        l, a = lax.fori_loop(0, NC, weigh, (jnp.zeros((1, TQ), F32), jnp.zeros((DH, TQ), F32)))
        ot[pl.ds(pl.multiple_of(h * DH, DH), DH), pl.ds(q0, TQ)] = a
        l8 = jnp.broadcast_to(l * 0.125, (8, TQ))
        for n in range(NCOL):
            lt[pl.ds(pl.multiple_of((j * NCOL + n) * LTR + h * 8, 8), 8), :] = l8[:, n * 128:(n + 1) * 128]
        return carry

    def wprep(r, carry):
        r16 = pl.multiple_of(r * 16, 16)
        r8 = pl.ds(pl.multiple_of(r * 8, 8), 8)

        def two(w, row, cols):
            return jnp.concatenate([w[pl.ds(r16 + row + e * 128, 16), cols].astype(F32) for e in range(2)], axis=0)

        for sc in range(NSC + 1):
            w_ = 256 if sc < NSC else 128
            cl = slice(sc * 256, sc * 256 + w_)
            cr = slice(HF + sc * 256, HF + sc * 256 + w_)
            rg, ru = [_rhs7(two(w, 0, cl), two(w, 0, cr), two(w, HD, cl), two(w, HD, cr)) for w in (wg, wu)]
            for i in range(7):
                if sc < NSC:
                    for m, (tg, tu) in enumerate(zip(_rhs7(*_quads(rg[i])), _rhs7(*_quads(ru[i])))):
                        wgu2[(sc * 7 + i) * 7 + m, r8, :] = _pk(jnp.concatenate([tg, tu], axis=1).astype(BF16))
                else:
                    t = _pk(jnp.concatenate([rg[i], ru[i]], axis=1).astype(BF16))
                    for e in range(2):
                        wgu1[i, e, r8, :] = t[e * 8:(e + 1) * 8]
        for sc in range(NSC):
            top, bot = two(wd, sc * 256, slice(None)), two(wd, HF + sc * 256, slice(None))
            for i, t in enumerate(_rhs7(top[:, :HD], top[:, HD:], bot[:, :HD], bot[:, HD:])):
                t7 = _pk(jnp.concatenate(_rhs7(*_quads(t)), axis=1).astype(BF16))
                for j in range(7):
                    wdn2[i * 7 + j, sc, r8, :] = t7[:, j * 128:(j + 1) * 128]
        top = wd[pl.ds(r16 + NSC * 256, 16), :].astype(F32)
        bot = wd[pl.ds(r16 + HF + NSC * 256, 16), :].astype(F32)
        for i, t in enumerate(_rhs7(top[:, :HD], top[:, HD:], bot[:, :HD], bot[:, HD:])):
            wdn1[i, r8, :] = _pk(t.astype(BF16))
        wop[pl.ds(pl.multiple_of(r * 32, 32), 32), :] = _pk(wo[pl.ds(pl.multiple_of(r * 64, 64), 64), :])
        return carry

    def o_tile(t):
        cols = pl.ds(_mult(t * TS, TS), TS)
        den = lt[pl.ds(t * LTR, H, stride=8), :]
        for i in range(1, 8):
            den = den + lt[pl.ds(t * LTR + i, H, stride=8), :]
        r = 1.0 / den
        o = jnp.concatenate([ot[h * DH:(h + 1) * DH, cols] * r[h:h + 1] for h in range(H)], axis=0)
        return o.T.astype(BF16)

    def o_stage(t):
        on[0] = _pk(o_tile(t))

    def ffn_pair(x1, xb, hs, gu_early, tie=False):
        zj = [zs[j] for j in range(8)]
        for s in range(NSUB):
            xb[s][0] = _ln(x1[s])
        la1 = [_lhs1(i, lambda q: xb[q // 2][zj[7], :, (q % 2) * HD:(q % 2 + 1) * HD]).astype(BF16)
               for i in range(7)]
        la2 = [[_lhs1(j, lambda r: _lhs1(i, lambda q: xb[q // 2][
            zj[j], (r // 2) * 64:(r // 2 + 1) * 64,
            (q % 2) * HD + (r % 2) * 128:(q % 2) * HD + (r % 2 + 1) * 128])).astype(BF16)
            for j in range(7)] for i in range(7)]

        def gu(i, sc, k):
            if sc == NSC:
                wi = wgu1[i].reshape(HD // 2, 256)
                if tie and i == GU_ORDER[-1]:
                    z = pltpu.bitcast(on[NSUB + zj[0], 0:8, 0:128], jnp.int32)
                    w0 = pltpu.bitcast(pltpu.bitcast(wi[:8, :128], jnp.int32) | z, F32)
                    wi = jnp.concatenate([jnp.concatenate([w0, wi[:8, 128:]], axis=1), wi[8:]], axis=0)
                return _mm(la1[i], _up(wi))
            return _join(_combine7({
                j: _mm(la2[i][j], _up(wgu2[(sc * 7 + i) * 7 + j, :, k * 128:(k + 1) * 128])) for j in IN_ORDER}))

        early = {(i, sc, k): gu(i, sc, k) for (sc, k) in gu_early for i in GU_ORDER[:2]}

        def outer(sc, k):
            return _combine7({i: early[(i, sc, k)] if (i, sc, k) in early else gu(i, sc, k) for i in GU_ORDER})

        for sc in range(NSC):
            for q, (g, u) in enumerate(zip(outer(sc, 0), outer(sc, 1))):
                hs[q, :, sc * 256:(sc + 1) * 256] = g * u
        hodd = [t[:, :128] * t[:, 128:] for t in outer(NSC, 0)]

        def dn_lhs(i, j):
            def blk(q, r):
                rows = slice((r // 2) * 64, (r // 2 + 1) * 64)
                return jnp.concatenate(
                    [hs[q + zj[j], rows, sc * 256 + (r % 2) * 128:sc * 256 + (r % 2 + 1) * 128]
                     for sc in range(NSC)], axis=1)
            return _lhs1(j, lambda r: _lhs1(i, lambda q: blk(q, r))).astype(BF16)

        m = {}
        for i in IN_ORDER:
            inner = {j: _mm(dn_lhs(i, j), _up(wdn2[i * 7 + j].reshape(NSC * 64, 128))) for j in IN_ORDER}
            m[i] = _join(_combine7(inner)) + _mm(_lhs1(i, lambda q: hodd[q]).astype(BF16), _up(wdn1[i]))
        c = _combine7(m)
        return [x1[s] + jnp.concatenate([c[2 * s], c[2 * s + 1]], axis=1) for s in range(NSUB)]

    def ffn_first(b, carry):
        rows = [pl.ds(pl.multiple_of(b * TB + s * TS, TS), TS) for s in range(NSUB)]
        o = [_up(on[0])] + [o_tile(b * NSUB + s) for s in range(1, NSUB)]
        x1 = [xin[rows[s], :].astype(F32) + _mm(o[s], _up(wop[...])) for s in range(NSUB)]
        o_stage(jnp.minimum(b + 1, NB - 1) * NSUB)
        x2 = ffn_pair(x1, (xb0, xb1), hs0, GU_EARLY)
        for s in range(NSUB):
            xs[rows[s], :] = x2[s]
        for s in range(NSUB):
            xn2 = _ln(x2[s]).astype(BF16)
            k_proj(xn2, b * NSUB + s)
            qv_proj(xn2, b * NSUB + s)
        return carry

    def ffn_last(i, carry):
        nt = 2 * NSUB
        rows = [pl.ds(pl.multiple_of((i * nt + s) * TS, TS), TS) for s in range(nt)]
        o = [_up(on[0])] + [o_tile(i * nt + s) for s in range(1, nt)]
        x1 = [xs[rows[s], :] + _mm(o[s], _up(wop[...])) for s in range(nt)]
        o_stage(jnp.minimum(i + 1, NB // 2 - 1) * nt)
        x2 = ffn_pair(x1[:NSUB], (xb0, xb1), hs0, (), tie=True) + ffn_pair(x1[NSUB:], (xb2, xb3), hs1, ())
        for s in range(nt):
            xin[rows[s], :] = x2[s].astype(BF16)
        for e in range(2):
            o_copy(2 * i + e).start()
        return carry

    def w_transpose(w, i):
        for j in range(4):
            wqvt[i * HD + j * 64:i * HD + (j + 1) * 64, :] = _pk(
                w[:, j * 128:(j + 1) * 128].astype(F32).T.astype(BF16))

    x_copy(0).start()
    wk_copy.start()
    zer[...] = jnp.zeros(zer.shape, zer.dtype)
    vsum[...] = jnp.zeros(vsum.shape, vsum.dtype)
    on[NSUB, 0:8, 0:128] = jnp.zeros((8, 128), F32)
    for n in range(8):
        zs[n] = 0
    x_copy(0).wait()
    wq_copy.start()
    ln_in(0)
    wk_copy.wait()
    wv_copy.start()
    x_copy(1).start()
    wkp[...] = _pk(wk[...])
    k_proj(_up(on[0]), 0)
    wq_copy.wait()
    k_proj(_up(on[1]), 1)
    w_transpose(wq, 0)
    q_store(_nt(_up(wqvt[:HD]), _up(on[0])), 0)
    wv_copy.wait()
    x_copy(1).wait()
    for b in range(2, NB):
        x_copy(b).start()
    q_store(_nt(_up(wqvt[:HD]), _up(on[1])), 1)
    w_transpose(wv, 1)
    for s in range(NSUB):
        v_store(_nt(_up(wqvt[HD:]), _up(on[s])), s)
    ln_in(1)
    for cp in w_copies:
        cp.start()
    lax.fori_loop(1, NB, qkv_block, 0)
    for cp in w_copies:
        cp.wait()
    lax.fori_loop(0, 8, wprep, 0)

    def layer(li, carry):
        chk[0] = jnp.zeros((8, TQ), F32)
        chk[1] = jnp.ones((8, TQ), F32)
        pc[...] = jnp.zeros(pc.shape, pc.dtype)
        ac[...] = jnp.zeros(ac.shape, ac.dtype)
        lc[...] = jnp.ones(lc.shape, lc.dtype)
        lax.fori_loop(0, H // NH, fast_step, 0)
        flush(H - 1)
        o_stage(0)

        vabs = jnp.concatenate([vsum[n * 8:(n + 1) * 8] for n in range(NCOL)], axis=1)
        ok = (chk[0] <= L_HI) & (chk[1] >= L_LO) & (vabs <= L_HI)

        @pl.when(jnp.max(jnp.where(ok, 0.0, 1.0)) > 0.0)
        def _():
            lax.fori_loop(0, H * NQ, safe_unit, 0)
            o_stage(0)

        @pl.when(li == 0)
        def _():
            lax.fori_loop(0, NB, ffn_first, 0)

        @pl.when(li == 1)
        def _():
            lax.fori_loop(0, NB // 2, ffn_last, 0)
        return carry

    lax.fori_loop(0, 2, layer, 0)
    for b in range(NB):
        o_copy(b).wait()


@jax.jit
def pallas_interleave_layers__softmax_full_mha__glu_gated_bilinear__prompt_kernel(
    A_x: jax.Array,
    A_wqkv: jax.Array,
    A_wo: jax.Array,
    B_x: jax.Array,
    B_w_gate: jax.Array,
    B_w_up: jax.Array,
    B_w_down: jax.Array,
):
    del B_x
    any_spec = pl.BlockSpec(memory_space=pl.ANY)
    out = pl.pallas_call(
        _kernel,
        out_shape=jax.ShapeDtypeStruct((S, D), A_x.dtype),
        in_specs=[any_spec] * 6,
        out_specs=any_spec,
        scratch_shapes=[
            pltpu.VMEM((S, D), BF16),
            pltpu.VMEM((D, D), BF16),
            pltpu.VMEM((D, D), BF16),
            pltpu.VMEM((D, D), BF16),
            pltpu.VMEM((D, D), BF16),
            pltpu.VMEM((D, F), BF16),
            pltpu.VMEM((D, F), BF16),
            pltpu.VMEM((F, D), BF16),
            pltpu.VMEM((HD, D), F32),
            pltpu.VMEM((HD, D), F32),
            pltpu.VMEM((7, 2, 64, 256), F32),
            pltpu.VMEM((NSC * 49, 64, 256), F32),
            pltpu.VMEM((7, 64, HD), F32),
            pltpu.VMEM((49, NSC, 64, 128), F32),
            pltpu.VMEM((S, D), F32),
            pltpu.VMEM((D, D), F32),
            pltpu.VMEM((4, S // 2, 128), F32),
            pltpu.VMEM((4, NVMAX, NC * 16, 128), F32),
            pltpu.VMEM((HD, S), F32),
            pltpu.VMEM((HD, S), F32),
            pltpu.VMEM((D, S), F32),
            pltpu.VMEM((NSUB + 1, TS // 2, D), F32),
            pltpu.VMEM((DH, TQ), F32),
            pltpu.VMEM((S // 2, 128), F32),
            pltpu.VMEM((S // 2, 128), F32),
            pltpu.VMEM((DH, KBG, 8, 128), F32),
            pltpu.VMEM((DH, KBG, 8, 128), F32),
            pltpu.VMEM((H, NC * DH, 1, 8, 128), F32),
            pltpu.VMEM((NC * LTR + 32, 128), F32),
            pltpu.VMEM((2, 8, TQ), F32),
            pltpu.VMEM((128, TQ), F32),
            pltpu.VMEM((DH, TQ), F32),
            pltpu.VMEM((8, TQ), F32),
            pltpu.VMEM((S, TQ), F32),
            pltpu.VMEM((32, 128), F32),
            pltpu.VMEM((4, TS, NSC * 256), F32),
            pltpu.VMEM((4, TS, NSC * 256), F32),
            pltpu.VMEM((1, TS, D), F32),
            pltpu.VMEM((1, TS, D), F32),
            pltpu.VMEM((1, TS, D), F32),
            pltpu.VMEM((1, TS, D), F32),
            pltpu.SMEM((8,), jnp.int32),
            pltpu.SemaphoreType.DMA((NB,)),
            pltpu.SemaphoreType.DMA((7,)),
            pltpu.SemaphoreType.DMA((NB,)),
        ],
        compiler_params=pltpu.CompilerParams(vmem_limit_bytes=110 * 1024 * 1024),
    )(A_x.reshape(S, D), A_wqkv, A_wo, B_w_gate, B_w_up, B_w_down)
    return out.reshape(1, S, D)
```

```python
import math

import jax
import jax.numpy as jnp
from jax import lax
import jax.experimental.pallas as pl
import jax.experimental.pallas.tpu as pltpu

S, D, H, DH, F = 2048, 512, 32, 16, 1792
EPS = 1e-5
QSCALE = (DH ** -0.5) * math.log2(math.e)
F32 = jnp.float32
BF16 = jnp.bfloat16

TB = 256
TS = 128
NSUB = TB // TS
NB = S // TB
HD = D // 2
HF = F // 2
NSC = HF // 256
GU_EARLY = ((0, 0), (0, 1), (3, 0))
GU_ORDER = (2, 4, 0, 3, 6, 1, 5)
IN_ORDER = (0, 3, 4, 6, 2, 1, 5)

TQ = 512
NQ = S // TQ
NCOL = TQ // 128
NC = S // 128
T = NQ * NC
NH = 2
TT = NH * T
OFF = 2
VPOS = (1, 2, 4, 6)
XGAPS = (3, 3, 3, 3, 4)
XPOS = (0, 3)
XSH = 2
PSTEP = 2
DG = 4
LTR = H * 8
L_LO = 2.0 ** -40
L_HI = 2.0 ** 60

NV = [1] * TT
XS = [[] for _ in range(TT + 1)]
_prev = XSH - 1
for _gap in XGAPS * (TT // sum(XGAPS)):
    _t = _prev + _gap
    if _t >= TT - 1:
        break
    NV[_t] += 1
    for _n in range(NCOL):
        for _x in range(2):
            XS[_prev + 1 + ((2 * _n + _x) * _gap) // (2 * NCOL)].append((_t, _n, NV[_t] - 1, XPOS[_x], (_x,)))
    _prev = _t
NVC = [max(NV[c::NC]) for c in range(NC)]
NVMAX = max(NVC)

XC = [c for c in range(NC) if NVC[c] > 1]
KBG = 2 * NC * NVMAX + 2


def _ln(x):
    mu = jnp.mean(x, axis=-1, keepdims=True)
    xc = x - mu
    var = jnp.mean(xc * xc, axis=-1, keepdims=True)
    return xc * lax.rsqrt(var + EPS)


def _pk(a):
    return pltpu.bitcast(a, F32)


def _up(a):
    return pltpu.bitcast(a, BF16)


def _mm(a, b):
    return lax.dot_general(a, b, (((1,), (0,)), ((), ())), preferred_element_type=F32)


def _nt(a, b):
    return lax.dot_general(a, b, (((1,), (1,)), ((), ())), preferred_element_type=F32)


def _lhs1(i, a):
    p, sign, q = ((0, 1, 3), (2, 1, 3), (0, 0, 0), (3, 0, 0), (0, 1, 1), (2, -1, 0), (1, -1, 3))[i]
    return a(p) if sign == 0 else (a(p) + a(q) if sign > 0 else a(p) - a(q))


def _rhs7(b11, b12, b21, b22):
    return [b11 + b22, b11, b12 - b22, b21 - b11, b22, b11 + b12, b21 + b22]


def _combine7(m):
    return (m[0] + m[3] - m[4] + m[6], m[2] + m[4], m[1] + m[3], m[0] - m[1] + m[2] + m[5])


def _quads(a):
    r, c = a.shape[0] // 2, a.shape[1] // 2
    return a[:r, :c], a[:r, c:], a[r:, :c], a[r:, c:]


def _join(c):
    return jnp.concatenate([jnp.concatenate(c[:2], axis=1), jnp.concatenate(c[2:], axis=1)], axis=0)


def _rev_blocks(a):
    return jnp.concatenate([a[(15 - i) * 8:(16 - i) * 8] for i in range(16)], axis=0)


def _mult(v, m):
    return v if isinstance(v, int) else pl.multiple_of(v, m)


def _kernel(x_hbm, wqkv_hbm, wo_hbm, wg_hbm, wu_hbm, wd_hbm, o_hbm,
            xin, wq, wk, wv, wo, wg, wu, wd, wkp, wop, wgu1, wgu2, wdn1, wdn2, xs, wqvt,
            kk, kv, qt, vt, ot, on, zer, kra, krb, kba, kbb, qe, lt, chk, pc, ac, lc, sbuf, vsum,
            hs0, hs1, xb0, xb1, xb2, xb3, zs, sem_x, sem_w, sem_o):
    def x_copy(b):
        return pltpu.make_async_copy(x_hbm.at[pl.ds(b * TB, TB)], xin.at[pl.ds(b * TB, TB)], sem_x.at[b])

    def o_copy(b):
        return pltpu.make_async_copy(xin.at[pl.ds(b * TB, TB)], o_hbm.at[pl.ds(b * TB, TB)], sem_o.at[b])

    w_copies = [pltpu.make_async_copy(src, dst, sem_w.at[i]) for i, (src, dst) in enumerate(
        [(wo_hbm, wo), (wg_hbm, wg), (wu_hbm, wu), (wd_hbm, wd)])]
    wq_copy, wk_copy, wv_copy = [
        pltpu.make_async_copy(wqkv_hbm.at[:, pl.ds(i * D, D)], dst, sem_w.at[4 + i])
        for i, dst in enumerate((wq, wk, wv))]

    def k_proj(xn, t):
        p0 = _mult(t * (TS // 2), TS // 2)
        k = _rev_blocks(_mm(xn, _up(wkp[...]))).astype(BF16)
        kf = k[0:NVMAX * 16].astype(F32)
        for g in range(4):
            kp = _pk(k[:, g * 128:(g + 1) * 128])
            kk[g, pl.ds(p0, TS // 2), :] = kp
            for b in range(NVMAX):
                kv[g, b, pl.ds(_mult(t * 16, 16), 16), :] = kf[b * 16:(b + 1) * 16, g * 128:(g + 1) * 128]
            if g == 0:
                kra[pl.ds(p0, TS // 2), :] = kp
        for b in range(NVMAX):
            for d in range(DH):
                kba[d, pl.ds(2 * (b * NC + t), 2)] = jnp.broadcast_to(
                    kf[b * 16:(b + 1) * 16, d:d + 1], (16, 128)).reshape(2, 8, 128)

    def q_store(qf, t):
        q = (qf * QSCALE).astype(BF16)
        qt[:, pl.ds(_mult(t * TS, TS), TS)] = _pk(q)
        qe[:, pl.ds(t * DH, DH)] = jnp.broadcast_to(
            q.astype(F32)[:, None, :], (D, 8, TS)).reshape(H, DH, 1, 8, TS)

    def v_store(v, t):
        vt[:, pl.ds(_mult(t * TS, TS), TS)] = _pk(v.astype(BF16))
        vsum[...] = vsum[...] + jnp.sum(jnp.abs(v).reshape(D // 32, 32, TS), axis=0)

    def qv_proj(xn, t):
        qv = _nt(_up(wqvt[...]), xn)
        q_store(qv[:D], t)
        v_store(qv[D:], t)

    def ln_in(b):
        for s in range(NSUB):
            r0 = _mult(b * TB + s * TS, TS)
            on[s] = _pk(_ln(xin[pl.ds(r0, TS), :].astype(F32)).astype(BF16))

    def qkv_block(b, carry):
        @pl.when(b + 1 < NB)
        def _():
            x_copy(b + 1).wait()
        for s in range(NSUB):
            k_proj(_up(on[s]), b * NSUB + s)
            qv_proj(_up(on[s]), b * NSUB + s)
        ln_in(jnp.minimum(b + 1, NB - 1))
        return carry

    def gather(x, idx):
        return jnp.take_along_axis(x, idx, axis=1, mode="promise_in_bounds")

    def prep_piece(h, kr, kb, d):
        g = lax.shift_right_logical(h, 3)
        lane0 = (h & 7) * DH
        rows = slice(d * 64, (d + 1) * 64)
        kr[rows, :] = gather(kk[g, rows, :], (lax.broadcasted_iota(jnp.int32, (64, 128), 1) + lane0) & 127)
        src = jnp.concatenate([kv[g, 0]] + [kv[g, 1, c * 16:(c + 1) * 16, :] for c in XC], axis=0)
        col = gather(src, jnp.full(src.shape, lane0 + d, jnp.int32)).reshape(-1, 8, 128)
        kb[d, 0:2 * NC] = col[0:2 * NC]
        for m, c in enumerate(XC):
            kb[d, 2 * (NC + c):2 * (NC + c) + 2] = col[2 * (NC + m):2 * (NC + m) + 2]

    def finish(h, j, a, l8):
        ot[pl.ds(_mult(h * DH, DH), DH), j * TQ:(j + 1) * TQ] = a
        for n in range(NCOL):
            lt[pl.ds(_mult((j * NCOL + n) * LTR + h * 8, 8), 8), :] = l8[:, n * 128:(n + 1) * 128]
        chk[0] = chk[0] + l8
        chk[1] = jnp.minimum(chk[1], l8)

    def flush(h):
        a = ac[...] + _mm(_up(vt[pl.ds(_mult(h * 8, 8), 8), S - 128:S]), pc[...])
        finish(h, NQ - 1, a, lc[...])

    def fast_step(i, carry):
        heads = [NH * i + k for k in range(NH)]
        krs, kbs = (kra, krb), (kba, kbb)
        r0 = [pl.multiple_of(h * 8, 8) for h in heads]
        pblk, lsum, acc, done, snap = {}, {}, {}, {}, {}
        zz = [zs[n] * 32 for n in range(NCOL + 1)]
        heads2 = [h + zs[NCOL + 1] for h in heads]

        def ladd(u, n, p):
            l = lsum.get((u, n))
            if l is None:
                l = zer[0:8, 0:128]
            lsum[(u, n)] = jnp.sum(jnp.concatenate([l[None], p], axis=0), axis=0)

        def vpu_part(t, n, b, halves):
            u, c = divmod(t, NC)
            k = t // T
            grp = pl.ds(2 * (b * NC + c) + halves[0] + zz[n], len(halves))
            hq = heads2[k] if b else heads[k]
            sv = None
            for d0 in range(0, DH, DG):
                row = ((u % NQ) * NCOL + n) * DH + d0
                q8 = qe[hq, row:row + DG]
                if t == TT - 1:
                    q8 = jnp.where(snap[n] < 0.0, 0.0, q8)
                pr = kbs[k][d0:d0 + DG, grp] * q8
                if sv is not None:
                    pr = jnp.concatenate([sv, pr], axis=0)
                sv = jnp.sum(pr, axis=0, keepdims=d0 + DG < DH)
            p = jnp.exp2(sv)
            ladd(u, n, p)
            if t == TT - 2:
                snap[n] = lsum[(u, n)]
            for m, x in enumerate(halves):
                pm = p[m:m + 1] if len(halves) > 1 else p
                pblk[(t, b, x, n)] = pm
                if u > 0 and not done.get(u - 1):
                    lsum[(u - 1, n)] = jnp.where(pm[0] < 0.0, pm[0], lsum[(u - 1, n)])

        def dot_blocks(blist, vsched):
            if not blist:
                return
            u = blist[0][0] // NC
            k, j = divmod(u, NQ)
            w = jnp.concatenate(
                [_up(qt[pl.ds(r0[k], 8), j * TQ:(j + 1) * TQ]), jnp.zeros((128 - DH, TQ), BF16)], axis=0)
            runs = {}
            for t, b in blist:
                runs.setdefault(t, []).append(b)
            kc = _up(jnp.concatenate(
                [krs[k][pl.ds(pl.multiple_of((t % NC) * 64 + bs[0] * 8 + zz[NCOL], 8), len(bs) * 8), :]
                 for t, bs in runs.items()], axis=0))
            p = jnp.exp2(_mm(kc, w)).reshape(2 * len(blist), 8, TQ)
            for m, (t, b) in enumerate(blist):
                for x in range(2):
                    pblk[(t, b, x)] = p[2 * m + x:2 * m + x + 1]
            first = [0] * NCOL

            def catch_up(n, m):
                if m > first[n]:
                    ladd(u, n, p[2 * first[n]:2 * m, :, n * 128:(n + 1) * 128])
                    first[n] = m

            for m in range(len(blist)):
                for part in vsched.pop(0):
                    catch_up(part[1], m)
                    vpu_part(*part)
            for n in range(NCOL):
                catch_up(n, len(blist))
            if blist[-1] == (u * NC + NC - 1, 7):
                done[u] = True

        def qk(t):
            l0 = [(t - 1, b) for b in range(NV[t - 1] + OFF, 8)] if t >= 1 else []
            l1 = [(t, b) for b in range(NV[t], NV[t] + OFF)] if t < TT else []
            nb = len(l0) + len(l1)
            vs = [[] for _ in range(nb)]
            parts = [(t, n, 0, VPOS[n], (0, 1)) for n in range(NCOL)] if t < TT else []
            for (tt, n, b, pos, halves) in parts + XS[t]:
                vs[min(pos, nb - 1)].append((tt, n, b, halves))
            if t % NC:
                dot_blocks(l0 + l1, vs)
            else:
                dot_blocks(l0, vs)
                dot_blocks(l1, vs)

        def ptile(t):
            return jnp.concatenate([
                pblk.pop((t, b, x)) if b >= NV[t] else
                jnp.concatenate([pblk.pop((t, b, x, n)) for n in range(NCOL)], axis=2)
                for b in reversed(range(8)) for x in (1, 0)], axis=0).reshape(128, TQ)

        def lrow(u):
            return jnp.concatenate([lsum[(u, n)] for n in range(NCOL)], axis=1)

        def pv(t):
            u, c = divmod(t, NC)
            k, j = divmod(u, NQ)
            a = acc.get(u)
            if a is None:
                a = zer[...]
            a = a + _mm(_up(vt[pl.ds(r0[k], 8), c * 128:(c + 1) * 128]), ptile(t))
            acc[u] = a
            if c == NC - 1:
                finish(heads[k], j, a, lrow(u))

        for t in range(TT + 1):
            qk(t)
            if t == 1:
                flush(jnp.maximum(heads[0] - 1, 0))
            if t >= 2:
                pv(t - 2)
            k, tl = divmod(t, T)
            if k < NH and tl % PSTEP == 0 and tl // PSTEP < DH:
                prep_piece(jnp.minimum(heads[k] + 1, H - 1), krs[1 - k], kbs[1 - k], tl // PSTEP)
        pc[...] = ptile(TT - 1)
        ac[...] = acc[NH * NQ - 1]
        lc[...] = lrow(NH * NQ - 1)
        return carry

    def safe_unit(u, carry):
        h = lax.shift_right_logical(u, 2)
        g = lax.shift_right_logical(h, 3)
        j = u & (NQ - 1)
        q0 = pl.multiple_of(j * TQ, TQ)
        rows = lax.broadcasted_iota(jnp.int32, (128, TQ), 0)
        qg = _up(qt[pl.ds(pl.multiple_of(g * 64, 64), 64), pl.ds(q0, TQ)]).astype(F32)
        w = jnp.where(lax.shift_right_logical(rows, 4) == (h & 7), qg, 0.0).astype(BF16)

        def scores(c, m):
            s = _rev_blocks(_mm(_up(kk[g, pl.ds(pl.multiple_of(c * 64, 64), 64), :]), w))
            sbuf[pl.ds(pl.multiple_of(c * 128, 128), 128), :] = s
            return jnp.maximum(m, jnp.max(s, axis=0, keepdims=True))

        m = lax.fori_loop(0, NC, scores, jnp.full((1, TQ), -jnp.inf, F32))

        def weigh(c, la):
            l, a = la
            c0 = pl.multiple_of(c * 128, 128)
            p = jnp.exp2(sbuf[pl.ds(c0, 128), :] - m)
            l = l + jnp.sum(p, axis=0, keepdims=True)
            a = a + _mm(_up(vt[pl.ds(pl.multiple_of(h * 8, 8), 8), pl.ds(c0, 128)]), p.astype(BF16))
            return l, a

        l, a = lax.fori_loop(0, NC, weigh, (jnp.zeros((1, TQ), F32), jnp.zeros((DH, TQ), F32)))
        ot[pl.ds(pl.multiple_of(h * DH, DH), DH), pl.ds(q0, TQ)] = a
        l8 = jnp.broadcast_to(l * 0.125, (8, TQ))
        for n in range(NCOL):
            lt[pl.ds(pl.multiple_of((j * NCOL + n) * LTR + h * 8, 8), 8), :] = l8[:, n * 128:(n + 1) * 128]
        return carry

    def wprep(r, carry):
        r16 = pl.multiple_of(r * 16, 16)
        r8 = pl.ds(pl.multiple_of(r * 8, 8), 8)

        def two(w, row, cols):
            return jnp.concatenate([w[pl.ds(r16 + row + e * 128, 16), cols].astype(F32) for e in range(2)], axis=0)

        for sc in range(NSC + 1):
            w_ = 256 if sc < NSC else 128
            cl = slice(sc * 256, sc * 256 + w_)
            cr = slice(HF + sc * 256, HF + sc * 256 + w_)
            rg, ru = [_rhs7(two(w, 0, cl), two(w, 0, cr), two(w, HD, cl), two(w, HD, cr)) for w in (wg, wu)]
            for i in range(7):
                if sc < NSC:
                    for m, (tg, tu) in enumerate(zip(_rhs7(*_quads(rg[i])), _rhs7(*_quads(ru[i])))):
                        wgu2[(sc * 7 + i) * 7 + m, r8, :] = _pk(jnp.concatenate([tg, tu], axis=1).astype(BF16))
                else:
                    t = _pk(jnp.concatenate([rg[i], ru[i]], axis=1).astype(BF16))
                    for e in range(2):
                        wgu1[i, e, r8, :] = t[e * 8:(e + 1) * 8]
        for sc in range(NSC):
            top, bot = two(wd, sc * 256, slice(None)), two(wd, HF + sc * 256, slice(None))
            for i, t in enumerate(_rhs7(top[:, :HD], top[:, HD:], bot[:, :HD], bot[:, HD:])):
                t7 = _pk(jnp.concatenate(_rhs7(*_quads(t)), axis=1).astype(BF16))
                for j in range(7):
                    wdn2[i * 7 + j, sc, r8, :] = t7[:, j * 128:(j + 1) * 128]
        top = wd[pl.ds(r16 + NSC * 256, 16), :].astype(F32)
        bot = wd[pl.ds(r16 + HF + NSC * 256, 16), :].astype(F32)
        for i, t in enumerate(_rhs7(top[:, :HD], top[:, HD:], bot[:, :HD], bot[:, HD:])):
            wdn1[i, r8, :] = _pk(t.astype(BF16))
        wop[pl.ds(pl.multiple_of(r * 32, 32), 32), :] = _pk(wo[pl.ds(pl.multiple_of(r * 64, 64), 64), :])
        return carry

    def o_tile(t):
        cols = pl.ds(_mult(t * TS, TS), TS)
        den = lt[pl.ds(t * LTR, H, stride=8), :]
        for i in range(1, 8):
            den = den + lt[pl.ds(t * LTR + i, H, stride=8), :]
        r = 1.0 / den
        o = jnp.concatenate([ot[h * DH:(h + 1) * DH, cols] * r[h:h + 1] for h in range(H)], axis=0)
        return o.T.astype(BF16)

    def o_stage(t):
        on[0] = _pk(o_tile(t))

    def ffn_pair(x1, xb, hs, gu_early, tie=False):
        zj = [zs[j] for j in range(8)]
        for s in range(NSUB):
            xb[s][0] = _ln(x1[s])
        la1 = [_lhs1(i, lambda q: xb[q // 2][zj[7], :, (q % 2) * HD:(q % 2 + 1) * HD]).astype(BF16)
               for i in range(7)]
        la2 = [[_lhs1(j, lambda r: _lhs1(i, lambda q: xb[q // 2][
            zj[j], (r // 2) * 64:(r // 2 + 1) * 64,
            (q % 2) * HD + (r % 2) * 128:(q % 2) * HD + (r % 2 + 1) * 128])).astype(BF16)
            for j in range(7)] for i in range(7)]

        def gu(i, sc, k):
            if sc == NSC:
                wi = wgu1[i].reshape(HD // 2, 256)
                if tie and i == GU_ORDER[-1]:
                    z = pltpu.bitcast(on[NSUB + zj[0], 0:8, 0:128], jnp.int32)
                    w0 = pltpu.bitcast(pltpu.bitcast(wi[:8, :128], jnp.int32) | z, F32)
                    wi = jnp.concatenate([jnp.concatenate([w0, wi[:8, 128:]], axis=1), wi[8:]], axis=0)
                return _mm(la1[i], _up(wi))
            return _join(_combine7({
                j: _mm(la2[i][j], _up(wgu2[(sc * 7 + i) * 7 + j, :, k * 128:(k + 1) * 128])) for j in IN_ORDER}))

        early = {(i, sc, k): gu(i, sc, k) for (sc, k) in gu_early for i in GU_ORDER[:2]}

        def outer(sc, k):
            return _combine7({i: early[(i, sc, k)] if (i, sc, k) in early else gu(i, sc, k) for i in GU_ORDER})

        for sc in range(NSC):
            for q, (g, u) in enumerate(zip(outer(sc, 0), outer(sc, 1))):
                hs[q, :, sc * 256:(sc + 1) * 256] = g * u
        hodd = [t[:, :128] * t[:, 128:] for t in outer(NSC, 0)]

        def dn_lhs(i, j):
            def blk(q, r):
                rows = slice((r // 2) * 64, (r // 2 + 1) * 64)
                return jnp.concatenate(
                    [hs[q + zj[j], rows, sc * 256 + (r % 2) * 128:sc * 256 + (r % 2 + 1) * 128]
                     for sc in range(NSC)], axis=1)
            return _lhs1(j, lambda r: _lhs1(i, lambda q: blk(q, r))).astype(BF16)

        m = {}
        for i in IN_ORDER:
            inner = {j: _mm(dn_lhs(i, j), _up(wdn2[i * 7 + j].reshape(NSC * 64, 128))) for j in IN_ORDER}
            m[i] = _join(_combine7(inner)) + _mm(_lhs1(i, lambda q: hodd[q]).astype(BF16), _up(wdn1[i]))
        c = _combine7(m)
        return [x1[s] + jnp.concatenate([c[2 * s], c[2 * s + 1]], axis=1) for s in range(NSUB)]

    def ffn_first(b, carry):
        rows = [pl.ds(pl.multiple_of(b * TB + s * TS, TS), TS) for s in range(NSUB)]
        o = [_up(on[0])] + [o_tile(b * NSUB + s) for s in range(1, NSUB)]
        x1 = [xin[rows[s], :].astype(F32) + _mm(o[s], _up(wop[...])) for s in range(NSUB)]
        o_stage(jnp.minimum(b + 1, NB - 1) * NSUB)
        x2 = ffn_pair(x1, (xb0, xb1), hs0, GU_EARLY)
        for s in range(NSUB):
            xs[rows[s], :] = x2[s]
        for s in range(NSUB):
            xn2 = _ln(x2[s]).astype(BF16)
            k_proj(xn2, b * NSUB + s)
            qv_proj(xn2, b * NSUB + s)
        return carry

    def ffn_last(i, carry):
        nt = 2 * NSUB
        rows = [pl.ds(pl.multiple_of((i * nt + s) * TS, TS), TS) for s in range(nt)]
        o = [_up(on[0])] + [o_tile(i * nt + s) for s in range(1, nt)]
        x1 = [xs[rows[s], :] + _mm(o[s], _up(wop[...])) for s in range(nt)]
        o_stage(jnp.minimum(i + 1, NB // 2 - 1) * nt)
        for e, (xb, hs) in enumerate((((xb0, xb1), hs0), ((xb2, xb3), hs1))):
            x2 = ffn_pair(x1[e * NSUB:(e + 1) * NSUB], xb, hs, (), tie=e == 0)
            for s in range(NSUB):
                xin[rows[e * NSUB + s], :] = x2[s].astype(BF16)
            o_copy(2 * i + e).start()
        return carry

    def w_transpose(w, i):
        for j in range(4):
            wqvt[i * HD + j * 64:i * HD + (j + 1) * 64, :] = _pk(
                w[:, j * 128:(j + 1) * 128].astype(F32).T.astype(BF16))

    x_copy(0).start()
    wk_copy.start()
    zer[...] = jnp.zeros(zer.shape, zer.dtype)
    vsum[...] = jnp.zeros(vsum.shape, vsum.dtype)
    on[NSUB, 0:8, 0:128] = jnp.zeros((8, 128), F32)
    for n in range(8):
        zs[n] = 0
    x_copy(0).wait()
    wq_copy.start()
    ln_in(0)
    wk_copy.wait()
    wv_copy.start()
    x_copy(1).start()
    wkp[...] = _pk(wk[...])
    k_proj(_up(on[0]), 0)
    wq_copy.wait()
    k_proj(_up(on[1]), 1)
    w_transpose(wq, 0)
    q_store(_nt(_up(wqvt[:HD]), _up(on[0])), 0)
    wv_copy.wait()
    x_copy(1).wait()
    for b in range(2, NB):
        x_copy(b).start()
    q_store(_nt(_up(wqvt[:HD]), _up(on[1])), 1)
    w_transpose(wv, 1)
    for s in range(NSUB):
        v_store(_nt(_up(wqvt[HD:]), _up(on[s])), s)
    ln_in(1)
    for cp in w_copies:
        cp.start()
    lax.fori_loop(1, NB, qkv_block, 0)
    for cp in w_copies:
        cp.wait()
    lax.fori_loop(0, 8, wprep, 0)

    def layer(li, carry):
        chk[0] = jnp.zeros((8, TQ), F32)
        chk[1] = jnp.ones((8, TQ), F32)
        pc[...] = jnp.zeros(pc.shape, pc.dtype)
        ac[...] = jnp.zeros(ac.shape, ac.dtype)
        lc[...] = jnp.ones(lc.shape, lc.dtype)
        lax.fori_loop(0, H // NH, fast_step, 0)
        flush(H - 1)
        o_stage(0)

        vabs = jnp.concatenate([vsum[n * 8:(n + 1) * 8] for n in range(NCOL)], axis=1)
        ok = (chk[0] <= L_HI) & (chk[1] >= L_LO) & (vabs <= L_HI)

        @pl.when(jnp.max(jnp.where(ok, 0.0, 1.0)) > 0.0)
        def _():
            lax.fori_loop(0, H * NQ, safe_unit, 0)
            o_stage(0)

        @pl.when(li == 0)
        def _():
            lax.fori_loop(0, NB, ffn_first, 0)

        @pl.when(li == 1)
        def _():
            lax.fori_loop(0, NB // 2, ffn_last, 0)
        return carry

    lax.fori_loop(0, 2, layer, 0)
    for b in range(NB):
        o_copy(b).wait()


@jax.jit
def pallas_interleave_layers__softmax_full_mha__glu_gated_bilinear__prompt_kernel(
    A_x: jax.Array,
    A_wqkv: jax.Array,
    A_wo: jax.Array,
    B_x: jax.Array,
    B_w_gate: jax.Array,
    B_w_up: jax.Array,
    B_w_down: jax.Array,
):
    del B_x
    any_spec = pl.BlockSpec(memory_space=pl.ANY)
    out = pl.pallas_call(
        _kernel,
        out_shape=jax.ShapeDtypeStruct((S, D), A_x.dtype),
        in_specs=[any_spec] * 6,
        out_specs=any_spec,
        scratch_shapes=[
            pltpu.VMEM((S, D), BF16),
            pltpu.VMEM((D, D), BF16),
            pltpu.VMEM((D, D), BF16),
            pltpu.VMEM((D, D), BF16),
            pltpu.VMEM((D, D), BF16),
            pltpu.VMEM((D, F), BF16),
            pltpu.VMEM((D, F), BF16),
            pltpu.VMEM((F, D), BF16),
            pltpu.VMEM((HD, D), F32),
            pltpu.VMEM((HD, D), F32),
            pltpu.VMEM((7, 2, 64, 256), F32),
            pltpu.VMEM((NSC * 49, 64, 256), F32),
            pltpu.VMEM((7, 64, HD), F32),
            pltpu.VMEM((49, NSC, 64, 128), F32),
            pltpu.VMEM((S, D), F32),
            pltpu.VMEM((D, D), F32),
            pltpu.VMEM((4, S // 2, 128), F32),
            pltpu.VMEM((4, NVMAX, NC * 16, 128), F32),
            pltpu.VMEM((HD, S), F32),
            pltpu.VMEM((HD, S), F32),
            pltpu.VMEM((D, S), F32),
            pltpu.VMEM((NSUB + 1, TS // 2, D), F32),
            pltpu.VMEM((DH, TQ), F32),
            pltpu.VMEM((S // 2, 128), F32),
            pltpu.VMEM((S // 2, 128), F32),
            pltpu.VMEM((DH, KBG, 8, 128), F32),
            pltpu.VMEM((DH, KBG, 8, 128), F32),
            pltpu.VMEM((H, NC * DH, 1, 8, 128), F32),
            pltpu.VMEM((NC * LTR + 32, 128), F32),
            pltpu.VMEM((2, 8, TQ), F32),
            pltpu.VMEM((128, TQ), F32),
            pltpu.VMEM((DH, TQ), F32),
            pltpu.VMEM((8, TQ), F32),
            pltpu.VMEM((S, TQ), F32),
            pltpu.VMEM((32, 128), F32),
            pltpu.VMEM((4, TS, NSC * 256), F32),
            pltpu.VMEM((4, TS, NSC * 256), F32),
            pltpu.VMEM((1, TS, D), F32),
            pltpu.VMEM((1, TS, D), F32),
            pltpu.VMEM((1, TS, D), F32),
            pltpu.VMEM((1, TS, D), F32),
            pltpu.SMEM((8,), jnp.int32),
            pltpu.SemaphoreType.DMA((NB,)),
            pltpu.SemaphoreType.DMA((7,)),
            pltpu.SemaphoreType.DMA((NB,)),
        ],
        compiler_params=pltpu.CompilerParams(vmem_limit_bytes=110 * 1024 * 1024),
    )(A_x.reshape(S, D), A_wqkv, A_wo, B_w_gate, B_w_up, B_w_down)
    return out.reshape(1, S, D)
```

```python
import math

import jax
import jax.numpy as jnp
from jax import lax
import jax.experimental.pallas as pl
import jax.experimental.pallas.tpu as pltpu

S, D, H, DH, F = 2048, 512, 32, 16, 1792
EPS = 1e-5
QSCALE = (DH ** -0.5) * math.log2(math.e)
F32 = jnp.float32
BF16 = jnp.bfloat16

TB = 256
TS = 128
NSUB = TB // TS
NB = S // TB
HD = D // 2
HF = F // 2
NSC = HF // 256
GU_EARLY = ((0, 0), (0, 1), (3, 0))
GU_ORDER = (2, 4, 0, 3, 6, 1, 5)
IN_ORDER = (0, 3, 4, 6, 2, 1, 5)
QVG = 32

TQ = 512
NQ = S // TQ
NCOL = TQ // 128
NC = S // 128
T = NQ * NC
NH = 2
TT = NH * T
OFF = 2
VPOS = (1, 3, 5, 6)
XGAPS = (3, 3, 3, 3, 4)
XPOS = (0, 4)
XSH = 2
PSTEP = 3
DG = 4
LTR = H * 8
L_LO = 2.0 ** -40
L_HI = 2.0 ** 60

NV = [1] * TT
XS = [[] for _ in range(TT + 1)]
_prev = XSH - 1
for _gap in XGAPS * (TT // sum(XGAPS)):
    _t = _prev + _gap
    if _t >= TT - 1:
        break
    NV[_t] += 1
    for _n in range(NCOL):
        for _x in range(2):
            XS[_prev + 1 + ((2 * _n + _x) * _gap) // (2 * NCOL)].append((_t, _n, NV[_t] - 1, XPOS[_x], (_x,)))
    _prev = _t
NVC = [max(NV[c::NC]) for c in range(NC)]
NVMAX = max(NVC)

XC = [c for c in range(NC) if NVC[c] > 1]
KBG = 2 * NC * NVMAX + 3


def _ln(x):
    mu = jnp.mean(x, axis=-1, keepdims=True)
    xc = x - mu
    var = jnp.mean(xc * xc, axis=-1, keepdims=True)
    return xc * lax.rsqrt(var + EPS)


def _pk(a):
    return pltpu.bitcast(a, F32)


def _up(a):
    return pltpu.bitcast(a, BF16)


def _mm(a, b):
    return lax.dot_general(a, b, (((1,), (0,)), ((), ())), preferred_element_type=F32)


def _nt(a, b):
    return lax.dot_general(a, b, (((1,), (1,)), ((), ())), preferred_element_type=F32)


def _lhs1(i, a):
    p, sign, q = ((0, 1, 3), (2, 1, 3), (0, 0, 0), (3, 0, 0), (0, 1, 1), (2, -1, 0), (1, -1, 3))[i]
    return a(p) if sign == 0 else (a(p) + a(q) if sign > 0 else a(p) - a(q))


def _rhs7(b11, b12, b21, b22):
    return [b11 + b22, b11, b12 - b22, b21 - b11, b22, b11 + b12, b21 + b22]


def _combine7(m):
    return (m[0] + m[3] - m[4] + m[6], m[2] + m[4], m[1] + m[3], m[0] - m[1] + m[2] + m[5])


def _quads(a):
    r, c = a.shape[0] // 2, a.shape[1] // 2
    return a[:r, :c], a[:r, c:], a[r:, :c], a[r:, c:]


def _join(c):
    return jnp.concatenate([jnp.concatenate(c[:2], axis=1), jnp.concatenate(c[2:], axis=1)], axis=0)


def _rev_blocks(a):
    return jnp.concatenate([a[(15 - i) * 8:(16 - i) * 8] for i in range(16)], axis=0)


def _mult(v, m):
    return v if isinstance(v, int) else pl.multiple_of(v, m)


def _kernel(x_hbm, wqkv_hbm, wo_hbm, wg_hbm, wu_hbm, wd_hbm, o_hbm,
            xin, wq, wk, wv, wo, wg, wu, wd, wkp, wop, wgu1, wgu2, wdn1, wdn2, xs, wqvt,
            kk, kv, qt, vt, ot, on, zer, kra, krb, kba, kbb, qe, lt, chk, pc, ac, lc, sbuf, vsum,
            hs0, hs1, xb0, xb1, xb2, xb3, zs, sem_x, sem_w, sem_o):
    def x_copy(b):
        return pltpu.make_async_copy(x_hbm.at[pl.ds(b * TB, TB)], xin.at[pl.ds(b * TB, TB)], sem_x.at[b])

    def o_copy(b):
        return pltpu.make_async_copy(xin.at[pl.ds(b * TB, TB)], o_hbm.at[pl.ds(b * TB, TB)], sem_o.at[b])

    w_copies = [pltpu.make_async_copy(src, dst, sem_w.at[i]) for i, (src, dst) in enumerate(
        [(wo_hbm, wo), (wg_hbm, wg), (wu_hbm, wu), (wd_hbm, wd)])]
    wq_copy, wk_copy, wv_copy = [
        pltpu.make_async_copy(wqkv_hbm.at[:, pl.ds(i * D, D)], dst, sem_w.at[4 + i])
        for i, dst in enumerate((wq, wk, wv))]

    def k_proj(xn, t):
        p0 = _mult(t * (TS // 2), TS // 2)
        k = _rev_blocks(_mm(xn, _up(wkp[...]))).astype(BF16)
        kf = k[0:NVMAX * 16].astype(F32)
        for g in range(4):
            kp = _pk(k[:, g * 128:(g + 1) * 128])
            kk[g, pl.ds(p0, TS // 2), :] = kp
            for b in range(NVMAX):
                kv[g, b, pl.ds(_mult(t * 16, 16), 16), :] = kf[b * 16:(b + 1) * 16, g * 128:(g + 1) * 128]
            if g == 0:
                kra[pl.ds(p0, TS // 2), :] = kp
        for b in range(NVMAX):
            for d in range(DH):
                kba[d, pl.ds(2 * (b * NC + t), 2)] = jnp.broadcast_to(
                    kf[b * 16:(b + 1) * 16, d:d + 1], (16, 128)).reshape(2, 8, 128)

    def q_store(qf, t):
        q = (qf * QSCALE).astype(BF16)
        qt[:, pl.ds(_mult(t * TS, TS), TS)] = _pk(q)
        qe[:, pl.ds(t * DH, DH)] = jnp.broadcast_to(
            q.astype(F32)[:, None, :], (D, 8, TS)).reshape(H, DH, 1, 8, TS)

    def v_store(v, t):
        vt[:, pl.ds(_mult(t * TS, TS), TS)] = _pk(v.astype(BF16))
        vsum[...] = vsum[...] + jnp.sum(jnp.abs(v).reshape(D // 32, 32, TS), axis=0)

    def qv_proj(xn, t):
        qv = _nt(_up(wqvt[...].reshape(D, D)), xn).reshape(D // QVG, 2, QVG, TS)
        q_store(qv[:, 0].reshape(D, TS), t)
        v_store(qv[:, 1].reshape(D, TS), t)

    def ln_in(b):
        for s in range(NSUB):
            r0 = _mult(b * TB + s * TS, TS)
            on[s] = _pk(_ln(xin[pl.ds(r0, TS), :].astype(F32)).astype(BF16))

    def qkv_block(b, carry):
        @pl.when(b + 1 < NB)
        def _():
            x_copy(b + 1).wait()
        for s in range(NSUB):
            k_proj(_up(on[s]), b * NSUB + s)
            qv_proj(_up(on[s]), b * NSUB + s)
        ln_in(jnp.minimum(b + 1, NB - 1))
        return carry

    def gather(x, idx):
        return jnp.take_along_axis(x, idx, axis=1, mode="promise_in_bounds")

    def prep_piece(h, kr, kb, d):
        g = lax.shift_right_logical(h, 3)
        lane0 = (h & 7) * DH
        rows = slice(d * 64, (d + 1) * 64)
        kr[rows, :] = gather(kk[g, rows, :], (lax.broadcasted_iota(jnp.int32, (64, 128), 1) + lane0) & 127)
        src = jnp.concatenate([kv[g, 0]] + [kv[g, 1, c * 16:(c + 1) * 16, :] for c in XC], axis=0)
        col = gather(src, jnp.full(src.shape, lane0 + d, jnp.int32)).reshape(-1, 8, 128)
        kb[d, 0:2 * NC] = col[0:2 * NC]
        for m, c in enumerate(XC):
            kb[d, 2 * (NC + c):2 * (NC + c) + 2] = col[2 * (NC + m):2 * (NC + m) + 2]

    def finish(h, j, a, l8):
        ot[pl.ds(_mult(h * DH, DH), DH), j * TQ:(j + 1) * TQ] = a
        for n in range(NCOL):
            lt[pl.ds(_mult((j * NCOL + n) * LTR + h * 8, 8), 8), :] = l8[:, n * 128:(n + 1) * 128]
        chk[0] = chk[0] + l8
        chk[1] = jnp.minimum(chk[1], l8)

    def flush(h):
        a = ac[...] + _mm(_up(vt[pl.ds(_mult(h * 8, 8), 8), S - 128:S]), pc[...])
        finish(h, NQ - 1, a, lc[...])

    def fast_step(i, carry):
        heads = [NH * i + k for k in range(NH)]
        krs, kbs = (kra, krb), (kba, kbb)
        r0 = [pl.multiple_of(h * 8, 8) for h in heads]
        pblk, lsum, acc, done, snap = {}, {}, {}, {}, {}
        zz = [zs[n] * 32 for n in range(NCOL + 1)]
        heads2 = [h + zs[NCOL + 1] for h in heads]

        def ladd(u, n, p):
            l = lsum.get((u, n))
            if l is None:
                l = zer[0:8, 0:128]
            lsum[(u, n)] = jnp.sum(jnp.concatenate([l[None], p], axis=0), axis=0)

        def vpu_part(t, n, b, halves):
            u, c = divmod(t, NC)
            k = t // T
            grp = pl.ds(2 * (b * NC + c) + halves[0] + zz[n], len(halves))
            hq = heads2[k] if b else heads[k]
            sv = None
            for d0 in range(0, DH, DG):
                row = ((u % NQ) * NCOL + n) * DH + d0
                q8 = qe[hq, row:row + DG]
                if t == TT - 1:
                    q8 = jnp.where(snap[n] < 0.0, 0.0, q8)
                pr = kbs[k][d0:d0 + DG, grp] * q8
                if sv is not None:
                    pr = jnp.concatenate([sv, pr], axis=0)
                sv = jnp.sum(pr, axis=0, keepdims=d0 + DG < DH)
            p = jnp.exp2(sv)
            ladd(u, n, p)
            if t == TT - 2:
                snap[n] = lsum[(u, n)]
            for m, x in enumerate(halves):
                pm = p[m:m + 1] if len(halves) > 1 else p
                pblk[(t, b, x, n)] = pm
                if u > 0 and not done.get(u - 1):
                    lsum[(u - 1, n)] = jnp.where(pm[0] < 0.0, pm[0], lsum[(u - 1, n)])

        def dot_blocks(blist, vsched):
            if not blist:
                return
            u = blist[0][0] // NC
            k, j = divmod(u, NQ)
            w = jnp.concatenate(
                [_up(qt[pl.ds(r0[k], 8), j * TQ:(j + 1) * TQ]), jnp.zeros((128 - DH, TQ), BF16)], axis=0)
            runs = {}
            for t, b in blist:
                runs.setdefault(t, []).append(b)
            kc = _up(jnp.concatenate(
                [krs[k][pl.ds(pl.multiple_of((t % NC) * 64 + bs[0] * 8 + zz[NCOL], 8), len(bs) * 8), :]
                 for t, bs in runs.items()], axis=0))
            p = jnp.exp2(_mm(kc, w)).reshape(2 * len(blist), 8, TQ)
            for m, (t, b) in enumerate(blist):
                for x in range(2):
                    pblk[(t, b, x)] = p[2 * m + x:2 * m + x + 1]
            first = [0] * NCOL

            def catch_up(n, m):
                if m > first[n]:
                    ladd(u, n, p[2 * first[n]:2 * m, :, n * 128:(n + 1) * 128])
                    first[n] = m

            for m in range(len(blist)):
                for part in vsched.pop(0):
                    catch_up(part[1], m)
                    vpu_part(*part)
            for n in range(NCOL):
                catch_up(n, len(blist))
            if blist[-1] == (u * NC + NC - 1, 7):
                done[u] = True

        def qk(t):
            l0 = [(t - 1, b) for b in range(NV[t - 1] + OFF, 8)] if t >= 1 else []
            l1 = [(t, b) for b in range(NV[t], NV[t] + OFF)] if t < TT else []
            nb = len(l0) + len(l1)
            vs = [[] for _ in range(nb)]
            parts = [(t, n, 0, VPOS[n], (0, 1)) for n in range(NCOL)] if t < TT else []
            for (tt, n, b, pos, halves) in parts + XS[t]:
                vs[min(pos, nb - 1)].append((tt, n, b, halves))
            if t % NC:
                dot_blocks(l0 + l1, vs)
            else:
                dot_blocks(l0, vs)
                dot_blocks(l1, vs)

        def ptile(t):
            return jnp.concatenate([
                pblk.pop((t, b, x)) if b >= NV[t] else
                jnp.concatenate([pblk.pop((t, b, x, n)) for n in range(NCOL)], axis=2)
                for b in reversed(range(8)) for x in (1, 0)], axis=0).reshape(128, TQ)

        def lrow(u):
            return jnp.concatenate([lsum[(u, n)] for n in range(NCOL)], axis=1)

        def pv(t):
            u, c = divmod(t, NC)
            k, j = divmod(u, NQ)
            a = acc.get(u)
            if a is None:
                a = zer[...]
            a = a + _mm(_up(vt[pl.ds(r0[k], 8), c * 128:(c + 1) * 128]), ptile(t))
            acc[u] = a
            if c == NC - 1:
                finish(heads[k], j, a, lrow(u))

        for t in range(TT + 1):
            qk(t)
            if t == 1:
                flush(jnp.maximum(heads[0] - 1, 0))
            if t >= 2:
                pv(t - 2)
            k, tl = divmod(t, T)
            if k < NH and tl % PSTEP == 0 and tl // PSTEP < DH:
                prep_piece(jnp.minimum(heads[k] + 1, H - 1), krs[1 - k], kbs[1 - k], tl // PSTEP)
        pc[...] = ptile(TT - 1)
        ac[...] = acc[NH * NQ - 1]
        lc[...] = lrow(NH * NQ - 1)
        return carry

    def safe_unit(u, carry):
        h = lax.shift_right_logical(u, 2)
        g = lax.shift_right_logical(h, 3)
        j = u & (NQ - 1)
        q0 = pl.multiple_of(j * TQ, TQ)
        rows = lax.broadcasted_iota(jnp.int32, (128, TQ), 0)
        qg = _up(qt[pl.ds(pl.multiple_of(g * 64, 64), 64), pl.ds(q0, TQ)]).astype(F32)
        w = jnp.where(lax.shift_right_logical(rows, 4) == (h & 7), qg, 0.0).astype(BF16)

        def scores(c, m):
            s = _rev_blocks(_mm(_up(kk[g, pl.ds(pl.multiple_of(c * 64, 64), 64), :]), w))
            sbuf[pl.ds(pl.multiple_of(c * 128, 128), 128), :] = s
            return jnp.maximum(m, jnp.max(s, axis=0, keepdims=True))

        m = lax.fori_loop(0, NC, scores, jnp.full((1, TQ), -jnp.inf, F32))

        def weigh(c, la):
            l, a = la
            c0 = pl.multiple_of(c * 128, 128)
            p = jnp.exp2(sbuf[pl.ds(c0, 128), :] - m)
            l = l + jnp.sum(p, axis=0, keepdims=True)
            a = a + _mm(_up(vt[pl.ds(pl.multiple_of(h * 8, 8), 8), pl.ds(c0, 128)]), p.astype(BF16))
            return l, a

        l, a = lax.fori_loop(0, NC, weigh, (jnp.zeros((1, TQ), F32), jnp.zeros((DH, TQ), F32)))
        ot[pl.ds(pl.multiple_of(h * DH, DH), DH), pl.ds(q0, TQ)] = a
        l8 = jnp.broadcast_to(l * 0.125, (8, TQ))
        for n in range(NCOL):
            lt[pl.ds(pl.multiple_of((j * NCOL + n) * LTR + h * 8, 8), 8), :] = l8[:, n * 128:(n + 1) * 128]
        return carry

    def wprep(r, carry):
        r16 = pl.multiple_of(r * 16, 16)
        r8 = pl.ds(pl.multiple_of(r * 8, 8), 8)

        def two(w, row, cols):
            return jnp.concatenate([w[pl.ds(r16 + row + e * 128, 16), cols].astype(F32) for e in range(2)], axis=0)

        for sc in range(NSC + 1):
            w_ = 256 if sc < NSC else 128
            cl = slice(sc * 256, sc * 256 + w_)
            cr = slice(HF + sc * 256, HF + sc * 256 + w_)
            rg, ru = [_rhs7(two(w, 0, cl), two(w, 0, cr), two(w, HD, cl), two(w, HD, cr)) for w in (wg, wu)]
            for i in range(7):
                if sc < NSC:
                    for m, (tg, tu) in enumerate(zip(_rhs7(*_quads(rg[i])), _rhs7(*_quads(ru[i])))):
                        wgu2[(sc * 7 + i) * 7 + m, r8, :] = _pk(jnp.concatenate([tg, tu], axis=1).astype(BF16))
                else:
                    t = _pk(jnp.concatenate([rg[i], ru[i]], axis=1).astype(BF16))
                    for e in range(2):
                        wgu1[i, e, r8, :] = t[e * 8:(e + 1) * 8]
        for sc in range(NSC):
            top, bot = two(wd, sc * 256, slice(None)), two(wd, HF + sc * 256, slice(None))
            for i, t in enumerate(_rhs7(top[:, :HD], top[:, HD:], bot[:, :HD], bot[:, HD:])):
                t7 = _pk(jnp.concatenate(_rhs7(*_quads(t)), axis=1).astype(BF16))
                for j in range(7):
                    wdn2[i * 7 + j, sc, r8, :] = t7[:, j * 128:(j + 1) * 128]
        top = wd[pl.ds(r16 + NSC * 256, 16), :].astype(F32)
        bot = wd[pl.ds(r16 + HF + NSC * 256, 16), :].astype(F32)
        for i, t in enumerate(_rhs7(top[:, :HD], top[:, HD:], bot[:, :HD], bot[:, HD:])):
            wdn1[i, r8, :] = _pk(t.astype(BF16))
        wop[pl.ds(pl.multiple_of(r * 32, 32), 32), :] = _pk(wo[pl.ds(pl.multiple_of(r * 64, 64), 64), :])
        return carry

    def o_tile(t):
        cols = pl.ds(_mult(t * TS, TS), TS)
        den = lt[pl.ds(t * LTR, H, stride=8), :]
        for i in range(1, 8):
            den = den + lt[pl.ds(t * LTR + i, H, stride=8), :]
        r = 1.0 / den
        o = jnp.concatenate([ot[h * DH:(h + 1) * DH, cols] * r[h:h + 1] for h in range(H)], axis=0)
        return o.T.astype(BF16)

    def o_stage(t):
        on[0] = _pk(o_tile(t))

    def ffn_pair(x1, xb, hs, gu_early, tie=False):
        zj = [zs[j] for j in range(8)]
        for s in range(NSUB):
            xb[s][0] = _ln(x1[s])
        la1 = [_lhs1(i, lambda q: xb[q // 2][zj[7], :, (q % 2) * HD:(q % 2 + 1) * HD]).astype(BF16)
               for i in range(7)]
        la2 = [[_lhs1(j, lambda r: _lhs1(i, lambda q: xb[q // 2][
            zj[j], (r // 2) * 64:(r // 2 + 1) * 64,
            (q % 2) * HD + (r % 2) * 128:(q % 2) * HD + (r % 2 + 1) * 128])).astype(BF16)
            for j in range(7)] for i in range(7)]

        def gu(i, sc, k):
            if sc == NSC:
                wi = wgu1[i].reshape(HD // 2, 256)
                if tie and i == GU_ORDER[-1]:
                    z = pltpu.bitcast(on[NSUB + zj[0], 0:8, 0:128], jnp.int32)
                    w0 = pltpu.bitcast(pltpu.bitcast(wi[:8, :128], jnp.int32) | z, F32)
                    wi = jnp.concatenate([jnp.concatenate([w0, wi[:8, 128:]], axis=1), wi[8:]], axis=0)
                return _mm(la1[i], _up(wi))
            return _join(_combine7({
                j: _mm(la2[i][j], _up(wgu2[(sc * 7 + i) * 7 + j, :, k * 128:(k + 1) * 128])) for j in IN_ORDER}))

        early = {(i, sc, k): gu(i, sc, k) for (sc, k) in gu_early for i in GU_ORDER[:2]}

        def outer(sc, k):
            return _combine7({i: early[(i, sc, k)] if (i, sc, k) in early else gu(i, sc, k) for i in GU_ORDER})

        for sc in range(NSC):
            for q, (g, u) in enumerate(zip(outer(sc, 0), outer(sc, 1))):
                hs[q, :, sc * 256:(sc + 1) * 256] = g * u
        hodd = [t[:, :128] * t[:, 128:] for t in outer(NSC, 0)]

        def dn_lhs(i, j):
            def blk(q, r):
                rows = slice((r // 2) * 64, (r // 2 + 1) * 64)
                return jnp.concatenate(
                    [hs[q + zj[j], rows, sc * 256 + (r % 2) * 128:sc * 256 + (r % 2 + 1) * 128]
                     for sc in range(NSC)], axis=1)
            return _lhs1(j, lambda r: _lhs1(i, lambda q: blk(q, r))).astype(BF16)

        m = {}
        for i in IN_ORDER:
            inner = {j: _mm(dn_lhs(i, j), _up(wdn2[i * 7 + j].reshape(NSC * 64, 128))) for j in IN_ORDER}
            m[i] = _join(_combine7(inner)) + _mm(_lhs1(i, lambda q: hodd[q]).astype(BF16), _up(wdn1[i]))
        c = _combine7(m)
        return [x1[s] + jnp.concatenate([c[2 * s], c[2 * s + 1]], axis=1) for s in range(NSUB)]

    def ffn_first(b, carry):
        rows = [pl.ds(pl.multiple_of(b * TB + s * TS, TS), TS) for s in range(NSUB)]
        o = [_up(on[0])] + [o_tile(b * NSUB + s) for s in range(1, NSUB)]
        x1 = [xin[rows[s], :].astype(F32) + _mm(o[s], _up(wop[...])) for s in range(NSUB)]
        o_stage(jnp.minimum(b + 1, NB - 1) * NSUB)
        x2 = ffn_pair(x1, (xb0, xb1), hs0, GU_EARLY)
        for s in range(NSUB):
            xs[rows[s], :] = x2[s]
        for s in range(NSUB):
            xn2 = _ln(x2[s]).astype(BF16)
            k_proj(xn2, b * NSUB + s)
            qv_proj(xn2, b * NSUB + s)
        return carry

    def ffn_last(i, carry):
        nt = 2 * NSUB
        rows = [pl.ds(pl.multiple_of((i * nt + s) * TS, TS), TS) for s in range(nt)]
        o = [_up(on[0])] + [o_tile(i * nt + s) for s in range(1, nt)]
        x1 = [xs[rows[s], :] + _mm(o[s], _up(wop[...])) for s in range(nt)]
        o_stage(jnp.minimum(i + 1, NB // 2 - 1) * nt)
        for e, (xb, hs) in enumerate((((xb0, xb1), hs0), ((xb2, xb3), hs1))):
            x2 = ffn_pair(x1[e * NSUB:(e + 1) * NSUB], xb, hs, (), tie=e == 0)
            for s in range(NSUB):
                xin[rows[e * NSUB + s], :] = x2[s].astype(BF16)
            o_copy(2 * i + e).start()
        return carry

    def w_transpose(w, i):
        for j in range(4):
            n = 128 // QVG
            wqvt[j * n:(j + 1) * n, i] = _pk(
                w[:, j * 128:(j + 1) * 128].astype(F32).T.astype(BF16)).reshape(n, QVG // 2, D)

    x_copy(0).start()
    wk_copy.start()
    zer[...] = jnp.zeros(zer.shape, zer.dtype)
    vsum[...] = jnp.zeros(vsum.shape, vsum.dtype)
    on[NSUB, 0:8, 0:128] = jnp.zeros((8, 128), F32)
    for n in range(8):
        zs[n] = 0
    x_copy(0).wait()
    wq_copy.start()
    ln_in(0)
    wk_copy.wait()
    wv_copy.start()
    x_copy(1).start()
    wkp[...] = _pk(wk[...])
    k_proj(_up(on[0]), 0)
    wq_copy.wait()
    k_proj(_up(on[1]), 1)
    w_transpose(wq, 0)
    q_store(_nt(_up(wqvt[:, 0].reshape(HD, D)), _up(on[0])), 0)
    wv_copy.wait()
    x_copy(1).wait()
    for b in range(2, NB):
        x_copy(b).start()
    q_store(_nt(_up(wqvt[:, 0].reshape(HD, D)), _up(on[1])), 1)
    w_transpose(wv, 1)
    for s in range(NSUB):
        v_store(_nt(_up(wqvt[:, 1].reshape(HD, D)), _up(on[s])), s)
    ln_in(1)
    for cp in w_copies:
        cp.start()
    lax.fori_loop(1, NB, qkv_block, 0)
    for cp in w_copies:
        cp.wait()
    lax.fori_loop(0, 8, wprep, 0)

    def layer(li, carry):
        chk[0] = jnp.zeros((8, TQ), F32)
        chk[1] = jnp.ones((8, TQ), F32)
        pc[...] = jnp.zeros(pc.shape, pc.dtype)
        ac[...] = jnp.zeros(ac.shape, ac.dtype)
        lc[...] = jnp.ones(lc.shape, lc.dtype)
        lax.fori_loop(0, H // NH, fast_step, 0)
        flush(H - 1)
        o_stage(0)

        vabs = jnp.concatenate([vsum[n * 8:(n + 1) * 8] for n in range(NCOL)], axis=1)
        ok = (chk[0] <= L_HI) & (chk[1] >= L_LO) & (vabs <= L_HI)

        @pl.when(jnp.max(jnp.where(ok, 0.0, 1.0)) > 0.0)
        def _():
            lax.fori_loop(0, H * NQ, safe_unit, 0)
            o_stage(0)

        @pl.when(li == 0)
        def _():
            lax.fori_loop(0, NB, ffn_first, 0)

        @pl.when(li == 1)
        def _():
            lax.fori_loop(0, NB // 2, ffn_last, 0)
        return carry

    lax.fori_loop(0, 2, layer, 0)
    for b in range(NB):
        o_copy(b).wait()


@jax.jit
def pallas_interleave_layers__softmax_full_mha__glu_gated_bilinear__prompt_kernel(
    A_x: jax.Array,
    A_wqkv: jax.Array,
    A_wo: jax.Array,
    B_x: jax.Array,
    B_w_gate: jax.Array,
    B_w_up: jax.Array,
    B_w_down: jax.Array,
):
    del B_x
    any_spec = pl.BlockSpec(memory_space=pl.ANY)
    out = pl.pallas_call(
        _kernel,
        out_shape=jax.ShapeDtypeStruct((S, D), A_x.dtype),
        in_specs=[any_spec] * 6,
        out_specs=any_spec,
        scratch_shapes=[
            pltpu.VMEM((S, D), BF16),
            pltpu.VMEM((D, D), BF16),
            pltpu.VMEM((D, D), BF16),
            pltpu.VMEM((D, D), BF16),
            pltpu.VMEM((D, D), BF16),
            pltpu.VMEM((D, F), BF16),
            pltpu.VMEM((D, F), BF16),
            pltpu.VMEM((F, D), BF16),
            pltpu.VMEM((HD, D), F32),
            pltpu.VMEM((HD, D), F32),
            pltpu.VMEM((7, 2, 64, 256), F32),
            pltpu.VMEM((NSC * 49, 64, 256), F32),
            pltpu.VMEM((7, 64, HD), F32),
            pltpu.VMEM((49, NSC, 64, 128), F32),
            pltpu.VMEM((S, D), F32),
            pltpu.VMEM((D // QVG, 2, QVG // 2, D), F32),
            pltpu.VMEM((4, S // 2, 128), F32),
            pltpu.VMEM((4, NVMAX, NC * 16, 128), F32),
            pltpu.VMEM((HD, S), F32),
            pltpu.VMEM((HD, S), F32),
            pltpu.VMEM((D, S), F32),
            pltpu.VMEM((NSUB + 1, TS // 2, D), F32),
            pltpu.VMEM((DH, TQ), F32),
            pltpu.VMEM((S // 2, 128), F32),
            pltpu.VMEM((S // 2, 128), F32),
            pltpu.VMEM((DH, KBG, 8, 128), F32),
            pltpu.VMEM((DH, KBG, 8, 128), F32),
            pltpu.VMEM((H, NC * DH, 1, 8, 128), F32),
            pltpu.VMEM((NC * LTR + 32, 128), F32),
            pltpu.VMEM((2, 8, TQ), F32),
            pltpu.VMEM((128, TQ), F32),
            pltpu.VMEM((DH, TQ), F32),
            pltpu.VMEM((8, TQ), F32),
            pltpu.VMEM((S, TQ), F32),
            pltpu.VMEM((32, 128), F32),
            pltpu.VMEM((4, TS, NSC * 256), F32),
            pltpu.VMEM((4, TS, NSC * 256), F32),
            pltpu.VMEM((1, TS, D), F32),
            pltpu.VMEM((1, TS, D), F32),
            pltpu.VMEM((1, TS, D), F32),
            pltpu.VMEM((1, TS, D), F32),
            pltpu.SMEM((8,), jnp.int32),
            pltpu.SemaphoreType.DMA((NB,)),
            pltpu.SemaphoreType.DMA((7,)),
            pltpu.SemaphoreType.DMA((NB,)),
        ],
        compiler_params=pltpu.CompilerParams(vmem_limit_bytes=110 * 1024 * 1024),
    )(A_x.reshape(S, D), A_wqkv, A_wo, B_w_gate, B_w_up, B_w_down)
    return out.reshape(1, S, D)
```
